```python
import jax
import jax.numpy as jnp

def _softmax(x, axis=-1):
    return jax.nn.softmax(x, axis=axis)
def _gelu(x):
    return jax.nn.gelu(x, approximate=True)
def _silu(x):
    return jax.nn.silu(x)
def _sigmoid(x):
    return jax.nn.sigmoid(x)
def _layernorm(x, axis=-1, eps=1e-5):
    m = jnp.mean(x, axis=axis, keepdims=True)
    v = jnp.var(x, axis=axis, keepdims=True)
    return (x - m) / jnp.sqrt(v + eps)
def _scatter_add(tgt, idx, src, axis=0):
    return tgt.at[idx].add(src)
def _segment_sum(src, seg, n):
    return jax.ops.segment_sum(src, seg, n)
class _Rng:
    def __init__(self, key):
        self._k = key
    def _next(self):
        self._k, sub = jax.random.split(self._k)
        return sub
    def normal(self, shape):
        return jax.random.normal(self._next(), shape, dtype=jnp.bfloat16)
    def randint(self, lo, hi, shape):
        return jax.random.randint(self._next(), shape, lo, hi, dtype=jnp.int32)
    def uniform(self, shape, lo=0.0, hi=1.0):
        return jax.random.uniform(self._next(), shape, jnp.bfloat16, lo, hi)
    def permutation(self, n):
        return jax.random.permutation(self._next(), n)


kernel_name = 'standalone__batchnorm__prompt'

def setup_inputs():
    _rng = _Rng(jax.random.key(int.from_bytes(__import__("os").urandom(4), "little")))
    _w = (lambda a: (lambda t: t.astype(jnp.bfloat16) if jnp.issubdtype(t.dtype, jnp.floating) else t)(jnp.asarray(a)))
    B, S, C = 2, 2048, 1024
    K = 3
    return {
        "x": _w((lambda *s: _rng.normal(s) * 0.05)(B, S, C)),
        "w": _w((lambda *s: _rng.normal(s) * 0.05)(K, C, C) * (1.0 / (K * C) ** 0.5)),
        "mean": _w((lambda *s: _rng.normal(s) * 0.05)(C) * 0.1),
        "var": _w(jnp.abs((lambda *s: _rng.normal(s) * 0.05)(C)) + 0.5),
        "g": _w((lambda *s: _rng.normal(s) * 0.05)(C) + 1.0),
        "b": _w((lambda *s: _rng.normal(s) * 0.05)(C) * 0.1),
    }

def reference(x, w, mean, var, g, b):
    K = 3
    P = K // 2
    S = x.shape[1]
    xp = jnp.pad(x, ((0, 0), (P, P), (0, 0)))
    y = sum(jnp.einsum('bsc,cd->bsd', xp[:, k:k + S, :], w[k]) for k in range(K))
    inv_std = 1.0 / jnp.sqrt(var + 1e-5)
    y = (y - mean) * (g * inv_std) + b
    return _silu(y)
```

```python
import jax, jax.numpy as jnp, functools, contextlib
import numpy as np
import jax.experimental.pallas as pl
import jax.experimental.pallas.tpu as pltpu

A = 2.0 / 3.0
Bp = 1.5
A2, B2 = A * A, Bp * Bp
C1 = 1.0 / (2 * A2 * (A2 - B2))
C3 = 1.0 / (2 * B2 * (B2 - A2))
F32 = jnp.float32
U32 = jnp.uint32
BF16 = jnp.bfloat16

def pack(a, b): return pltpu.pack_elementwise([a, b], packed_dtype=BF16)
def bf(u): return pltpu.bitcast(u, BF16)
def mm(a, b): return jnp.dot(a, b, preferred_element_type=F32)

def bt(d0, d1, d2, d3, d4, d5):
    a2d2, b2d2, a2d3, b2d3 = A2 * d2, B2 * d2, A2 * d3, B2 * d3
    p = d4 - b2d2
    r = d4 - a2d2
    t = d1 - b2d3
    q = d1 - a2d3
    v0 = (d0 - a2d2) + p
    v5 = (d5 - a2d3) + t
    bq = Bp * q
    at = A * t
    return v0, p - bq, p + bq, r - at, r + at, v5

def make(RB=8, EB=32, WB=8, oprio=1, scopes=False, lastsplit=4, x1wait=2, opaque=True, c1bar=True):
    scope = jax.named_scope if scopes else (lambda n: contextlib.nullcontext())
    @jax.jit
    def f(x, w, mean, var, g, b):
        B, S, C = x.shape
        assert B == 2
        NC = C // 128
        Mt = S // 4
        PAD = 16
        XR = B * (S + PAD) + PAD
        KH = C // 2

        def kern(x_hbm, w_hbm, m_hbm, v_hbm, g_hbm, b_hbm, o_hbm,
                 xs, osb, wk, acc, pm, pv_, pg, pb, zs, zs2, xsem, wsem, osem, psem, *bufs):
            ug = bufs[0:3]; uh = bufs[3:3 + NC]; v0s = bufs[3 + NC:3 + 2 * NC]; v1s = bufs[3 + 2 * NC:3 + 3 * NC]
            KG = {0: (0, 0), 1: (1, 64), 2: (2, 128), 3: (2, 128)}
            def u_ref(j, i, r0):
                k = r0 // 64
                if k >= 4: return uh[j].at[i], r0 - 256
                gi, base = KG[k]
                return ug[gi].at[j, i], r0 - base
            def u_load(j, i, k0, k1):
                parts = []
                for (a, e) in ((0, 1), (1, 2), (2, 4), (4, 8)):
                    if k0 <= a and e <= k1:
                        ref, _ = u_ref(j, i, a * 64)
                        parts.append(ref[...])
                return bf(parts[0] if len(parts) == 1 else jnp.concatenate(parts, axis=0))
            def v_load(vs, i, k0, k1, m0=0, m1=Mt):
                parts = [vs[c][i, m0 // 2:m1 // 2, :] for c in range(k0, k1)]
                return bf(parts[0] if len(parts) == 1 else jnp.concatenate(parts, axis=1))
            zoff = []
            def xcopy(bb, c, s):
                return pltpu.make_async_copy(
                    x_hbm.at[bb, :, pl.ds(c * 128, 128)],
                    xs.at[c, pl.ds(PAD + bb * (S + PAD), S), :], xsem.at[s])
            def wcopy(k0, k1, s):
                return pltpu.make_async_copy(w_hbm.at[:, pl.ds(k0 * 128, (k1 - k0) * 128), :],
                                             wk.at[:, pl.ds(k0 * 128, (k1 - k0) * 128), :], wsem.at[s])
            def ocopy(bb, c, r0=0, n=S):
                return pltpu.make_async_copy(
                    osb.at[c, pl.ds(bb * S + r0, n), :],
                    o_hbm.at[bb, pl.ds(r0, n), pl.ds(c * 128, 128)], osem.at[0])
            par = (pm, pv_, pg, pb)
            pcopies = [pltpu.make_async_copy(r, par[i], psem.at[0]) for i, r in enumerate((m_hbm, v_hbm, g_hbm, b_hbm))]
            zcopy = pltpu.make_async_copy(zs, zs2, psem.at[1])

            xcopy(0, 0, 0).start(); wcopy(0, 1, 0).start()
            xcopy(0, 1, 1).start(); wcopy(1, 2, 1).start()
            zs[...] = jnp.zeros((8, 128), U32)
            zcopy.start()
            for p in pcopies: p.start()
            for c in range(NC):
                for k in range(B + 1):
                    xs[c, pl.ds(k * (S + PAD), PAD), :] = jnp.zeros((PAD, 128), BF16)
            xs32 = xs.bitcast(U32)
            os32 = osb.bitcast(U32)

            def unpackers(gv, n):
                if gv is None:
                    lo = lambda u: pltpu.bitcast(u << 16, F32)
                    hi = lambda u: pltpu.bitcast(u & jnp.uint32(0xFFFF0000), F32)
                    return lo, hi
                pred, val = gv
                gu = pltpu.bitcast(val, U32)
                mk = jnp.where(pred, jnp.uint32(0xFFFF0000), gu)
                sa = jnp.where(pred, jnp.uint32(16), gu)
                if n > 8:
                    mk = jnp.concatenate([mk] * (n // 8), axis=0); sa = jnp.concatenate([sa] * (n // 8), axis=0)
                lo = lambda u: pltpu.bitcast(u << sa, F32)
                hi = lambda u: pltpu.bitcast(u & mk, F32)
                return lo, hi

            def w_item(j, r0, gv):
                lo, hi = unpackers(gv, WB)
                raw = [pltpu.bitcast(wk[k, pl.ds(2 * r0, 2 * WB), pl.ds(j * 128, 128)], U32) for k in range(3)]
                res = []
                for un in (lo, hi):
                    w0, w1, w2 = (un(u) for u in raw)
                    e1 = C1 * w0 + (C1 * A2) * w2; o1 = (C1 * A) * w1
                    e3 = C3 * w0 + (C3 * B2) * w2; o3 = (C3 * Bp) * w1
                    res.append((e1 + o1, e1 - o1, e3 + o3, e3 - o3))
                vals = [raw[0]] + [pack(res[0][i], res[1][i]) for i in range(4)] + [raw[2]]
                for i in range(6):
                    ref, lr = u_ref(j, i, r0)
                    ref[pl.ds(pl.multiple_of(zoff[0] + lr, 8), WB), :] = vals[i]
            def w_items(js, k0, k1):
                return [functools.partial(w_item, j, r0) for j in js for r0 in range(k0 * 64, k1 * 64, WB)]

            def x_item(view, c, vdst, r0, gv):
                lo, hi = unpackers(gv, RB)
                u = [view[pl.ds(8 + 4 * r0 + o, RB, stride=4), :] for o in range(-1, 5)]
                e = [hi(u[0]), lo(u[1]), hi(u[1]), lo(u[2]), hi(u[2]), lo(u[3]), hi(u[3]), lo(u[4]), hi(u[4]), lo(u[5])]
                ve = bt(*e[0:6]); vo = bt(*e[4:10])
                for i in range(6):
                    vdst[c][i, pl.ds(pl.multiple_of(zoff[0] + r0, 8), RB), :] = pack(ve[i], vo[i])
            def x_items(bb, cs, vdst):
                base = (PAD + bb * (S + PAD)) // 2
                out = []
                for c in cs:
                    view = xs32.at[c, pl.ds(base - 8, S // 2 + 16), :]
                    out += [functools.partial(x_item, view, c, vdst, r0) for r0 in range(0, Mt // 2, RB)]
                return out

            def place(items, gates, f0, f1):
                pred = zs2[...] == 0
                for k, it in enumerate(items):
                    gi = min(int(len(gates) * (f0 + (f1 - f0) * k / len(items))), len(gates) - 1)
                    arr, r = gates[gi]
                    it((pred, arr[r:r + 8, 0:128]))

            def dot_a(i, k0, k1, raw=False):
                lhs = v_load(v0s, i, k0, k1)
                gw = 4 // (k1 - k0)
                gates = []
                for j0 in range(0, NC, gw):
                    cols = slice(j0 * 128, (j0 + gw) * 128)
                    if raw:
                        rhs = wk[0 if i == 0 else 2, k0 * 128:k1 * 128, cols]
                    else:
                        rhs = jnp.concatenate([u_load(j, i, k0, k1) for j in range(j0, j0 + gw)], axis=1)
                    r = mm(lhs, rhs)
                    if k0 > 0: r = acc[i, :, cols] + r
                    acc[i, :, cols] = r
                    gates += [(r, rr) for rr in range(0, Mt, 8)]
                return gates

            def epilogue(M, bb, c, m0, m1):
                sc, sh = bn
                scj, shj = sc[:, c * 128:(c + 1) * 128], sh[:, c * 128:(c + 1) * 128]
                ov = os32.at[c, pl.ds(bb * (S // 2), S // 2), :]
                for r0 in range(0, m1 - m0, EB):
                    m = [q[r0:r0 + EB] for q in M]
                    s1, d1, s2, d2 = m[1] + m[2], m[1] - m[2], m[3] + m[4], m[3] - m[4]
                    y = [m[0] + s1 + s2, A * d1 + Bp * d2, A2 * s1 + B2 * s2, (A2 * A) * d1 + (B2 * Bp) * d2 + m[5]]
                    o = []
                    for yy in y:
                        hh = yy * scj + shj
                        o.append(hh * jnp.tanh(hh) + hh)
                    ov[pl.ds(2 * (m0 + r0), EB, stride=2), :] = pack(o[0], o[1])
                    ov[pl.ds(2 * (m0 + r0) + 1, EB, stride=2), :] = pack(o[2], o[3])
                ocopy(bb, c, 4 * m0, 4 * (m1 - m0)).start(priority=oprio)

            allj = range(NC)
            with scope('w_x0'):
                xcopy(0, 0, 0).wait()
                zcopy.wait()
            zoff.append(zs2[0, 0].astype(jnp.int32) if opaque else 0)
            xcopy(0, 2, 2).start(); wcopy(2, 3, 2).start()
            xcopy(0, 3, 2).start(); wcopy(3, 4, 2).start()
            with scope('T0'):
                for it in x_items(0, [0], v0s): it(None)
            with scope('w_k0'):
                wcopy(0, 1, 0).wait()
            for c in range(4, 8): xcopy(0, c, 3).start()
            with scope('s0'):
                gt = dot_a(0, 0, 1, raw=True) + dot_a(5, 0, 1, raw=True)
                place(w_items(allj, 0, 1), gt, 0.0, 0.8)
                dot_a(1, 0, 1); dot_a(2, 0, 1)
            with scope('w_k1'):
                xcopy(0, 1, 1).wait(); wcopy(1, 2, 1).wait()
                for p in pcopies: p.wait()
            wcopy(4, 8, 3).start()
            with scope('s1'):
                pv = [par[i][...].astype(F32).reshape(1, C) for i in range(4)]
                sc = pv[2] * jax.lax.rsqrt(pv[1] + 1e-5)
                bn = (0.5 * sc, 0.5 * (pv[3] - pv[0] * sc))
                gt = dot_a(3, 0, 1) + dot_a(4, 0, 1)
                place(x_items(0, [1], v0s), gt, 0.0, 0.4)
                place(w_items(allj, 1, 2), gt, 0.3, 1.0)
                dot_a(0, 1, 2); dot_a(5, 1, 2); dot_a(1, 1, 2); dot_a(2, 1, 2)
            with scope('w_k23'):
                xcopy(0, 2, 2).wait(); xcopy(0, 3, 2).wait(); wcopy(2, 3, 2).wait(); wcopy(3, 4, 2).wait()
            for c in range(NC): xcopy(1, c, 4).start()
            with scope('s2'):
                gt = dot_a(3, 1, 2) + dot_a(4, 1, 2)
                place(x_items(0, [2, 3], v0s), gt, 0.0, 0.9)
                gt = dot_a(0, 2, 4, raw=True) + dot_a(5, 2, 4, raw=True)
                place(w_items(allj, 2, 4), gt, 0.0, 0.9)
                dot_a(1, 2, 4); dot_a(2, 2, 4)
            with scope('w_k47'):
                for c in range(4, 8): xcopy(0, c, 3).wait()
                wcopy(4, 8, 3).wait()
            with scope('s3'):
                gt = dot_a(3, 2, 4) + dot_a(4, 2, 4)
                place(x_items(0, [4, 5, 6, 7], v0s), gt, 0.0, 0.9)
                place(w_items([0], 4, 8), gt, 0.0, 0.9)
                xi = x_items(1, allj, v1s)
                nx = len(xi)
                for j in range(NC):
                    if j == x1wait:
                        with scope('w_x1'):
                            for c in range(NC): xcopy(1, c, 4).wait()
                    M = []; gt = []
                    for i in range(6):
                        q = acc[i, :, j * 128:(j + 1) * 128] + mm(v_load(v0s, i, 4, 8), u_load(j, i, 4, 8))
                        M.append(q); gt += [(q, r) for r in range(0, Mt, 8)]
                    if j + 1 < NC: place(w_items([j + 1], 4, 8), gt, 0.0, 0.8)
                    if j >= x1wait:
                        n0 = nx * (j - x1wait) // (NC - x1wait); n1 = nx * (j + 1 - x1wait) // (NC - x1wait)
                        place(xi[n0:n1], gt, 0.0, 0.85)
                    epilogue(M, 0, j, 0, Mt)
            with scope('w_c1'):
                if c1bar: ocopy(0, 0).wait()
            with scope('c1'):
                for j in range(NC):
                    ns = lastsplit if j == NC - 1 else 1
                    for sp in range(ns):
                        m0, m1 = sp * Mt // ns, (sp + 1) * Mt // ns
                        M = []
                        for i in range(6):
                            M.append(mm(v_load(v1s, i, 0, 8, m0, m1), u_load(j, i, 0, 8)))
                        epilogue(M, 1, j, m0, m1)
            with scope('w_out'):
                for c in range(1 if c1bar else 0, NC): ocopy(0, c).wait()
                for c in range(NC): ocopy(1, c).wait()

        anyspec = pl.BlockSpec(memory_space=pl.ANY)
        return pl.pallas_call(
            kern,
            in_specs=[anyspec] * 6,
            out_specs=anyspec,
            out_shape=jax.ShapeDtypeStruct(x.shape, x.dtype),
            scratch_shapes=[
                pltpu.VMEM((NC, XR, 128), BF16),
                pltpu.VMEM((NC, B * S, 128), BF16),
                pltpu.VMEM((3, C, C), BF16),
                pltpu.VMEM((6, Mt, C), F32),
                pltpu.VMEM((C,), BF16),
                pltpu.VMEM((C,), BF16),
                pltpu.VMEM((C,), BF16),
                pltpu.VMEM((C,), BF16),
                pltpu.VMEM((8, 128), U32),
                pltpu.VMEM((8, 128), U32),
                pltpu.SemaphoreType.DMA((5,)),
                pltpu.SemaphoreType.DMA((4,)),
                pltpu.SemaphoreType.DMA((1,)),
                pltpu.SemaphoreType.DMA((2,)),
                pltpu.VMEM((NC, 6, 64, 128), U32), pltpu.VMEM((NC, 6, 64, 128), U32), pltpu.VMEM((NC, 6, 128, 128), U32),
            ] + [pltpu.VMEM((6, 256, 128), U32)] * NC + [pltpu.VMEM((6, Mt // 2, 128), U32)] * (2 * NC),
            compiler_params=pltpu.CompilerParams(vmem_limit_bytes=110 * 2**20),
        )(x, w, mean, var, g, b)
    return f


pallas_standalone__batchnorm__prompt_kernel = make(c1bar=False, x1wait=3, lastsplit=8)
```

```python
import jax, jax.numpy as jnp, functools, contextlib
import jax.experimental.pallas as pl
import jax.experimental.pallas.tpu as pltpu

F32 = jnp.float32
U32 = jnp.uint32
BF16 = jnp.bfloat16

def pack(a, b): return pltpu.pack_elementwise([a, b], packed_dtype=BF16)
def bf(u): return pltpu.bitcast(u, BF16)
def mm(a, b): return jnp.dot(a, b, preferred_element_type=F32)
def cat(parts, axis): return parts[0] if len(parts) == 1 else jnp.concatenate(parts, axis=axis)


def make(PA=0.55, EB=16, oprio=1, scopes=False, lastsplit=(176, 96, 48, 32), order=(1, 2, 3, 4, 5, 6, 0, 7),
         skip=(6,), pf=(0.0, 0.95), w0free=12, s0n=3, s1n=5, s2n=3, g1=3, xa=(2, 0), xb=(5, 0), nxa=2, odelay=5, t2free=3, s2w=(0.25, 1.0), t2e=0.85, s1t=0.9, s1w=(0.3, 0.95), gate5=True, MA=160, wfree2=0, tb=(0.0, 0.5), wb=(0.2, 0.9)):
    scope = jax.named_scope if scopes else (lambda n: contextlib.nullcontext())
    a = PA; b = 1.0 / PA
    a2, b2 = a * a, b * b
    E = a2 + 1.0 + b2
    SS = a2 + b2
    c1 = 1.0 / (2.0 * (1.0 - a2) * (1.0 - b2))
    ca = 1.0 / (2.0 * a2 * (a2 - 1.0) * (a2 - b2))
    cb = 1.0 / (2.0 * b2 * (b2 - 1.0) * (b2 - a2))
    NP = 8

    def bt(d0, d1, d2, d3, d4, d5, d6, d7):
        d64, d42, d53, d31 = d6 - d4, d4 - d2, d5 - d3, d3 - d1
        v0 = (d0 - d6) + E * d42
        v7 = (d7 - d1) - E * d53
        e1 = (d6 + d2) - SS * d4
        o1 = (d5 + d1) - SS * d3
        ea = d64 - b2 * d42
        eb = d64 - a2 * d42
        oa = a * d53 - b * d31
        ob = b * d53 - a * d31
        return v0, e1 + o1, e1 - o1, ea + oa, ea - oa, eb + ob, eb - ob, v7

    def gt_(w0, w1, w2):
        e1 = c1 * (w0 + w2); o1 = c1 * w1
        ea = ca * w0 + (ca * a2) * w2; oa = (ca * a) * w1
        eb = cb * w0 + (cb * b2) * w2; ob = (cb * b) * w1
        return e1 + o1, e1 - o1, ea + oa, ea - oa, eb + ob, eb - ob

    @jax.jit
    def f(x, w, mean, var, g, b_):
        B, S, C = x.shape
        assert (B, S, C) == (2, 2048, 1024)
        NC = C // 128
        KH = C // 2
        PADF, GAP = 16, 8
        MT = (336, 352)
        T0 = (0, MT[0])
        NT = sum(MT)
        XR = PADF + 6 * NT + 24
        OR = 6 * NT + 16
        B1 = S + GAP

        def kern(x_hbm, w_hbm, m_hbm, v_hbm, g_hbm, b_hbm, o_hbm,
                 xs, osb, wl, wh, acc, pm, pv_, pg, pb, zs, zs2, zs3, zs4, xsem, wsem, osem, psem, *bufs):
            ug = bufs[0:5]; uh = bufs[5:5 + NC]; vs = (bufs[5 + NC:5 + 2 * NC], bufs[5 + 2 * NC:5 + 3 * NC]); va0 = bufs[5 + 3 * NC]
            xs32 = xs.bitcast(U32)
            os32 = osb.bitcast(U32)
            wh32 = wh.bitcast(U32)
            def u_ref(j, i, r0):
                k = r0 // 64
                if k >= 4: return uh[j].at[i - 1], r0 - 256
                if k == 0: return ug[j // 4].at[j % 4, i - 1], r0
                if k == 1: return ug[2].at[j, i - 1], r0 - 64
                return ug[3 + j // 4].at[j % 4, i - 1], r0 - 128
            def u_load(j0, j1, i, k0, k1):
                if i in (0, 7):
                    t = 0 if i == 0 else 2
                    if k0 >= 4: return bf(cat([wh32[j, t] for j in range(j0, j1)], 1))
                    return wl[t, k0 * 128:k1 * 128, j0 * 128:j1 * 128]
                return bf(cat([cat([u_ref(j, i, p * 64)[0][...] for (p, e) in ((0, 1), (1, 2), (2, 4), (4, 8))
                                    if k0 <= p and e <= k1], 0) for j in range(j0, j1)], 1))
            def v_load(ch, i, k0, k1, m0=0, m1=None):
                m1 = MT[ch] if m1 is None else m1
                return bf(cat([vs[ch][c][i, m0 // 2:m1 // 2, :] for c in range(k0, k1)], 1))
            zoff = []

            def xcopy(bb, c, s):
                return pltpu.make_async_copy(x_hbm.at[bb, :, pl.ds(c * 128, 128)],
                                             xs.at[c, pl.ds(PADF + bb * B1, S), :], xsem.at[s])
            def wcopy(k, s):
                return pltpu.make_async_copy(w_hbm.at[:, pl.ds(k * 128, 128), :], wl.at[:, pl.ds(k * 128, 128), :], wsem.at[s])
            def wtap(t, s):
                return pltpu.make_async_copy(w_hbm.at[t, pl.ds(0, 128), :], wl.at[t, pl.ds(0, 128), :], wsem.at[s])
            def whis(j0, j1, s):
                return [pltpu.make_async_copy(w_hbm.at[t, pl.ds(KH, KH), pl.ds(j * 128, 128)], wh.at[j, t], wsem.at[s])
                        for j in range(j0, j1) for t in range(3)]
            def ocopy1(bb, c, r0, n):
                return pltpu.make_async_copy(osb.at[c, pl.ds(bb * B1 + r0, n), :],
                                             o_hbm.at[bb, pl.ds(r0, n), pl.ds(c * 128, 128)], osem.at[0])
            def ocopies(c, q0, q1):
                out = []
                for bb in range(2):
                    lo_, hi_ = max(q0, bb * B1), min(q1, bb * B1 + S)
                    if hi_ > lo_: out.append(ocopy1(bb, c, lo_ - bb * B1, hi_ - lo_))
                return out
            par = (pm, pv_, pg, pb)
            pcopies = [pltpu.make_async_copy(r, par[i], psem.at[0]) for i, r in enumerate((m_hbm, v_hbm, g_hbm, b_hbm))]
            zcopy = pltpu.make_async_copy(zs, zs2, psem.at[1])
            def start(cs):
                for c in cs: c.start()
            def wait(cs):
                for c in cs: c.wait()
            g_k1 = [xcopy(0, 1, 1), wcopy(1, 1)]
            g_k23 = [xcopy(0, 2, 2), wcopy(2, 2), xcopy(0, 3, 2), wcopy(3, 2)]
            g_x47 = [xcopy(0, c, 3) for c in range(4, 8)]
            g_h1 = whis(0, g1, 3)
            g_h2 = whis(g1, NC, 0)
            g_xa = [xcopy(1, c, 4) for c in range(nxa)]
            g_xb = [xcopy(1, c, 0) for c in range(nxa, 8)]

            RA = 6 * MA + 16
            def xpart(r0, n, s):
                return pltpu.make_async_copy(x_hbm.at[0, pl.ds(r0, n), pl.ds(0, 128)], xs.at[0, pl.ds(PADF + r0, n), :], xsem.at[s])
            def wq(t, h, s):
                return pltpu.make_async_copy(w_hbm.at[t, pl.ds(0, 128), pl.ds(h * KH, KH)],
                                             wl.at[t, pl.ds(0, 128), pl.ds(h * KH, KH)], wsem.at[s])
            g_w1 = [wq(t, 0, 4) for t in range(3)]
            g_xa0 = [xpart(0, RA, 0)]
            g_w2 = [wq(t, 1, 5) for t in range(3)] + [xpart(RA, S - RA, 5)]
            zs[...] = jnp.zeros((8, 128), U32)
            start(g_w1)
            zcopy.start()
            start(g_xa0)
            zcopy2 = pltpu.make_async_copy(zs, zs3, psem.at[2])
            zcopy2.start()
            start(g_w2)
            zcopy3 = pltpu.make_async_copy(zs, zs4, psem.at[3])
            zcopy3.start()
            start(g_k1)
            for c in range(NC):
                for r0, n in ((0, PADF), (PADF + S, GAP), (PADF + B1 + S, XR - (PADF + B1 + S))):
                    xs[c, pl.ds(r0, n), :] = jnp.zeros((n, 128), BF16)

            def unpackers(gv):
                if gv is None:
                    lo = lambda u: pltpu.bitcast(u << 16, F32)
                    hi = lambda u: pltpu.bitcast(u & jnp.uint32(0xFFFF0000), F32)
                    return lo, hi
                pred, val = gv
                gu = pltpu.bitcast(val, U32)
                mk = jnp.where(pred, jnp.uint32(0xFFFF0000), gu)
                sa = jnp.where(pred, jnp.uint32(16), gu)
                lo = lambda u: pltpu.bitcast(u << sa, F32)
                hi = lambda u: pltpu.bitcast(u & mk, F32)
                return lo, hi

            def w_item(j, r0, gv):
                lo, hi = unpackers(gv)
                if r0 >= 256:
                    raw = [wh32[j, k, pl.ds(r0 - 256, 8), :] for k in range(3)]
                else:
                    raw = [pltpu.bitcast(wl[k, pl.ds(2 * r0, 16), pl.ds(j * 128, 128)], U32) for k in range(3)]
                ul = gt_(*(lo(u) for u in raw)); uh_ = gt_(*(hi(u) for u in raw))
                for i in range(1, 7):
                    ref, lr = u_ref(j, i, r0)
                    ref[pl.ds(pl.multiple_of(zoff[0] + lr, 8), 8), :] = pack(ul[i - 1], uh_[i - 1])
            def w_items(js, k0, k1):
                return [functools.partial(w_item, j, r0) for j in js for r0 in range(k0 * 64, k1 * 64, 8)]

            def x_item(ch, c, r0, gv):
                lo, hi = unpackers(gv)
                base = PADF // 2 + 3 * T0[ch] + 6 * r0
                u = [xs32[c, pl.ds(base + o, 8, stride=6), :] for o in range(-1, 7)]
                e = [hi(u[0])]
                for o in range(1, 7): e += [lo(u[o]), hi(u[o])]
                e.append(lo(u[7]))
                ve = bt(*e[0:8]); vo = bt(*e[6:14])
                dst = va0 if (ch == 0 and c == 0 and r0 < MA // 2) else vs[ch][c]
                for i in range(NP):
                    dst[i, pl.ds(pl.multiple_of(zoff[0] + r0, 8), 8), :] = pack(ve[i], vo[i])
            def x_items(ch, cs):
                return [functools.partial(x_item, ch, c, r0) for c in cs for r0 in range(0, MT[ch] // 2, 8)]

            def place(items, gates, f0, f1):
                pred = zs2[...] == 0
                for k, it in enumerate(items):
                    gi = min(int(len(gates) * (f0 + (f1 - f0) * k / len(items))), len(gates) - 1)
                    arr, r = gates[gi]
                    it((pred, arr[r:r + 8, 0:128]))

            def dot_a(i, k0, k1, ja=0, jb=NC):
                lhs = v_load(0, i, k0, k1)
                gw = 4 // (k1 - k0)
                gates = []
                for j0 in range(ja, jb, gw):
                    cols = slice(j0 * 128, (j0 + gw) * 128)
                    r = mm(lhs, u_load(j0, j0 + gw, i, k0, k1))
                    if k0 > 0: r = acc[i, 0:MT[0], cols] + r
                    acc[i, 0:MT[0], cols] = r
                    gates += [(r, rr) for rr in range(0, MT[0], 8)]
                return gates
            def dots_a(idx, k0, k1, ja=0, jb=NC):
                return sum((dot_a(i, k0, k1, ja, jb) for i in idx), [])

            def epilogue(M, ch, c, m0, m1, send=True):
                sc, sh = bn
                scj, shj = sc[:, c * 128:(c + 1) * 128], sh[:, c * 128:(c + 1) * 128]
                ka = [scj] + [(a ** k) * scj for k in range(1, 6)]
                kb = [scj] + [(b ** k) * scj for k in range(1, 6)]
                for r0 in range(0, m1 - m0, EB):
                    m = [q[r0:r0 + EB] for q in M]
                    p1 = ((m[1] + m[2]) * scj + shj, (m[1] - m[2]) * scj + shj)
                    pa = (m[3] + m[4], m[3] - m[4]); pb_ = (m[5] + m[6], m[5] - m[6])
                    kk = list(ka)
                    if gate5:
                        pred = zs2[...] == 0
                        for k in (1, 3, 5):
                            gk = jnp.where(pred, jnp.broadcast_to(ka[k], (8, 128)), m[5][0:8])
                            kk[k] = cat([gk] * (EB // 8), 0)
                    hs = [(p1[k % 2] + pa[k % 2] * kk[k]) + pb_[k % 2] * kb[k] for k in range(6)]
                    hs[0] = hs[0] + m[0] * scj
                    hs[5] = hs[5] + m[7] * scj
                    o = [hh * jnp.tanh(hh) + hh for hh in hs]
                    for p in range(3):
                        os32[c, pl.ds(3 * (T0[ch] + m0 + r0) + p, EB, stride=3), :] = pack(o[2 * p], o[2 * p + 1])
                if send:
                    for cp in ocopies(c, 6 * (T0[ch] + m0), 6 * (T0[ch] + m1)): cp.start(priority=oprio)

            allj = range(NC)
            def dot_0(i, part, h):
                m0, m1 = (0, MA) if part == 0 else (MA, MT[0])
                lhs = bf(va0[i]) if part == 0 else v_load(0, i, 0, 1, m0, m1)
                r = mm(lhs, u_load(4 * h, 4 * h + 4, i, 0, 1))
                acc[i, m0:m1, h * KH:(h + 1) * KH] = r
                return [(r, rr) for rr in range(0, m1 - m0, 8)]
            def dots_0(idx, part, h):
                return sum((dot_0(i, part, h) for i in idx), [])
            with scope('w_w1'):
                wait(g_w1)
                zcopy.wait(); zcopy2.wait(); zcopy3.wait()
            zoff.append(zs2[0, 0].astype(jnp.int32))
            with scope('W1'):
                start(pcopies); start(g_k23)
                for it in w_items(range(4), 0, 1): it(None)
            with scope('w_xa0'):
                wait(g_xa0)
            x0 = x_items(0, [0])
            with scope('S2'):
                for it in x0[:MA // 16]: it(None)
                dots_0(range(NP), 0, 0)
            with scope('w_w2'):
                wait(g_w2)
            with scope('s0'):
                gt = dots_0((0, 7), 0, 1)
                xb0 = x0[MA // 16:]
                for it in xb0[:3]: it(None)
                place(xb0[3:], gt, tb[0], tb[1])
                gt = gt + dots_0(range(NP), 1, 0)
                place(w_items(range(4, 8), 0, 1), gt, wb[0], wb[1])
                dots_0((0, 7), 1, 1)
                for i in range(1, s0n + 1): dots_0((i,), 0, 1); dots_0((i,), 1, 1)
                start(g_x47)
            with scope('w_k1'):
                wait(g_k1)
            with scope('s1'):
                gt = []
                for i in range(s0n + 1, 7): gt += dots_0((i,), 0, 1) + dots_0((i,), 1, 1)
                place(x_items(0, [1]), gt, 0.0, s1t)
                gt += dots_a((0, 7), 1, 2)
                place(w_items(allj, 1, 2), gt, s1w[0], s1w[1])
                dots_a(range(1, s1n + 1), 1, 2)
                start(g_h1)
            with scope('w_k23'):
                wait(g_k23); wait(pcopies)
            with scope('s2'):
                pv = [par[i][...].astype(F32).reshape(1, C) for i in range(4)]
                sc = pv[2] * jax.lax.rsqrt(pv[1] + 1e-5)
                bn = (0.5 * sc, 0.5 * (pv[3] - pv[0] * sc))
                gt = dots_a(range(s1n + 1, 7), 1, 2)
                x2 = x_items(0, [2])
                for it in x2[:t2free]: it(None)
                place(x2[t2free:], gt, 0.0, t2e)
                gt = dots_a((0, 7), 2, 3)
                place(x_items(0, [3]), gt, 0.0, 0.9)
                gt = gt + dots_a((0, 7), 3, 4)
                place(w_items(range(4), 2, 4), gt, s2w[0], s2w[1])
                gt = dots_a(range(1, s2n + 1), 2, 4, 0, 4)
                place(w_items(range(4, 8), 2, 4), gt, 0.0, 0.9)
                dots_a(range(1, s2n + 1), 2, 4, 4, 8)
                start(g_h2); start(g_xa)
            with scope('w_k47'):
                wait(g_x47); wait(g_h1)

            def block_b(ch, j, m0, m1, hooks):
                M = [None] * NP; gt = []
                for n_, i in enumerate(order):
                    if n_ in hooks:
                        hooks[n_](); gt = []
                    q = acc[i, m0:m1, j * 128:(j + 1) * 128] + mm(v_load(ch, i, 4, 8, m0, m1), u_load(j, j + 1, i, 4, 8))
                    M[i] = q
                    if i not in skip: gt += [(q, r) for r in range(0, m1 - m0, 8)]
                return M, gt
            def wait_a():
                with scope('w_xa'):
                    wait(g_xa); wait(g_h2)
                    if xb == xa: wait(g_xb)
            def wait_b():
                with scope('w_xb'):
                    wait(g_xb)
            with scope('s3'):
                gt = dots_a(range(s2n + 1, 7), 2, 4)
                start(g_xb)
                place(x_items(0, [4, 5, 6, 7]), gt, 0.0, 0.9)
                place(w_items([0], 4, 8), gt, 0.0, 0.9)
                def spread(items, p0, p1):
                    wts = [0.0] * NC
                    for j in range(p0[0], min(p1[0], NC)): wts[j] = 1.0 - (p0[1] / NP if j == p0[0] else 0.0)
                    cum = [sum(wts[:j]) / sum(wts) for j in range(NC + 1)]
                    return [items[int(len(items) * cum[j]):int(len(items) * cum[j + 1])] for j in range(NC)]
                if nxa >= 4 or xa == xb:
                    xi = spread(x_items(1, range(4)), xa, (NC, 0))
                else:
                    xi = [p + q for p, q in zip(spread(x_items(1, range(nxa)), xa, xb), spread(x_items(1, range(nxa, 4)), xb, (NC, 0)))]
                for j in range(NC):
                    hooks = {}
                    if j == xa[0]: hooks[xa[1]] = wait_a
                    if j == xb[0] and xb != xa: hooks[xb[1]] = wait_b
                    if odelay and j == odelay:
                        for jj in range(odelay):
                            for cp in ocopies(jj, 0, 6 * MT[0]): cp.start(priority=oprio)
                    M, gt = block_b(0, j, 0, MT[0], hooks)
                    if j + 1 < NC: place(w_items([j + 1], 4, 8), gt, pf[0], pf[1])
                    its = xi[j]
                    if its: place(its, gt, pf[0], pf[1])
                    epilogue(M, 0, j, 0, MT[0], send=not (j < odelay))
            with scope('c1a'):
                gt = []
                for j in range(NC):
                    for i in range(NP):
                        if xb != xa and (NC + j, i) == xb:
                            wait_b(); gt = []
                        q = mm(v_load(1, i, 0, 4), u_load(j, j + 1, i, 0, 4))
                        acc[i, :, j * 128:(j + 1) * 128] = q
                        gt += [(q, r) for r in range(0, MT[1], 8)]
                place(x_items(1, range(4, 8)), gt, 0.05, 0.9)
            with scope('c1b'):
                for j in range(NC):
                    m0 = 0
                    for n in (lastsplit if j == NC - 1 else (MT[1],)):
                        M, _ = block_b(1, j, m0, m0 + n, {})
                        epilogue(M, 1, j, m0, m0 + n)
                        m0 += n
            with scope('w_out'):
                for bb in range(2):
                    for c in range(NC): ocopy1(bb, c, 0, S).wait()

        anyspec = pl.BlockSpec(memory_space=pl.ANY)
        return pl.pallas_call(
            kern,
            in_specs=[anyspec] * 6,
            out_specs=anyspec,
            out_shape=jax.ShapeDtypeStruct(x.shape, x.dtype),
            scratch_shapes=[
                pltpu.VMEM((NC, XR, 128), BF16),
                pltpu.VMEM((NC, OR, 128), BF16),
                pltpu.VMEM((3, KH, C), BF16),
                pltpu.VMEM((NC, 3, KH, 128), BF16),
                pltpu.VMEM((NP, MT[1], C), F32),
                pltpu.VMEM((C,), BF16), pltpu.VMEM((C,), BF16), pltpu.VMEM((C,), BF16), pltpu.VMEM((C,), BF16),
                pltpu.VMEM((8, 128), U32), pltpu.VMEM((8, 128), U32),
                pltpu.VMEM((8, 128), U32), pltpu.VMEM((8, 128), U32),
                pltpu.SemaphoreType.DMA((6,)),
                pltpu.SemaphoreType.DMA((7,)),
                pltpu.SemaphoreType.DMA((1,)),
                pltpu.SemaphoreType.DMA((4,)),
                pltpu.VMEM((NC // 2, 6, 64, 128), U32), pltpu.VMEM((NC // 2, 6, 64, 128), U32),
                pltpu.VMEM((NC, 6, 64, 128), U32), pltpu.VMEM((NC // 2, 6, 128, 128), U32), pltpu.VMEM((NC // 2, 6, 128, 128), U32),
            ] + [pltpu.VMEM((6, 256, 128), U32)] * NC + [pltpu.VMEM((NP, MT[0] // 2, 128), U32)] * NC
              + [pltpu.VMEM((NP, MT[1] // 2, 128), U32)] * NC + [pltpu.VMEM((NP, MA // 2, 128), U32)],
            compiler_params=pltpu.CompilerParams(vmem_limit_bytes=110 * 2**20),
        )(x, w, mean, var, g, b_)
    return f


_impl = make(t2free=5, t2e=0.65, s2w=(0.2, 0.85))


@jax.jit
def pallas_standalone__batchnorm__prompt_kernel(x, w, mean, var, g, b):
    return _impl(x, w, mean, var, g, b)
```

```python
import jax, jax.numpy as jnp, functools, contextlib
import jax.experimental.pallas as pl
import jax.experimental.pallas.tpu as pltpu

F32 = jnp.float32
U32 = jnp.uint32
BF16 = jnp.bfloat16

def bf(u): return pltpu.bitcast(u, BF16)
def mm(a, b): return jnp.dot(a, b, preferred_element_type=F32)
def cat(parts, axis): return parts[0] if len(parts) == 1 else jnp.concatenate(parts, axis=axis)


def make(PA=0.55, oprio=1, scopes=False, lastsplit=(192, 96, 48, 16), order=(1, 2, 3, 4, 5, 6, 0, 7),
         skip=(6, 0), pf=(0.0, 0.9), s0n=4, s1n=5, s2n=4, g1=2, xa=(1, 1), xb=(4, 1), nxa=1, t3e=0.9, s3n=(0.45, 0.9),
         odelay=5, t2free=7, s2w=(0.4, 0.9), t2e=0.5, dgx=2, s1t=0.6, s1w=(0.2, 0.8), MA=192,
         tb=(0.0, 0.2), wb=(0.2, 0.9), phased=True, lag=2, oflag=True, omode='half', defer=False, ssa0=True, wsplit=2):
    scope = jax.named_scope if scopes else (lambda n: contextlib.nullcontext())
    a = PA; b = 1.0 / PA
    a2, b2 = a * a, b * b
    E = a2 + 1.0 + b2
    SS = a2 + b2
    c1 = 1.0 / (2.0 * (1.0 - a2) * (1.0 - b2))
    ca = 1.0 / (2.0 * a2 * (a2 - 1.0) * (a2 - b2))
    cb = 1.0 / (2.0 * b2 * (b2 - 1.0) * (b2 - a2))
    NP = 8

    def bt(d0, d1, d2, d3, d4, d5, d6, d7):
        d64, d42, d53, d31 = d6 - d4, d4 - d2, d5 - d3, d3 - d1
        v0 = (d0 - d6) + E * d42
        v7 = (d7 - d1) - E * d53
        e1 = (d6 + d2) - SS * d4
        o1 = (d5 + d1) - SS * d3
        ea = d64 - b2 * d42
        eb = d64 - a2 * d42
        oa = a * d53 - b * d31
        ob = b * d53 - a * d31
        return v0, e1 + o1, e1 - o1, ea + oa, ea - oa, eb + ob, eb - ob, v7

    def gt_(w0, w1, w2):
        e1 = c1 * (w0 + w2); o1 = c1 * w1
        ea = ca * w0 + (ca * a2) * w2; oa = (ca * a) * w1
        eb = cb * w0 + (cb * b2) * w2; ob = (cb * b) * w1
        return e1 + o1, e1 - o1, ea + oa, ea - oa, eb + ob, eb - ob

    @jax.jit
    def f(x, w, mean, var, g, b_):
        B, S, C = x.shape
        assert (B, S, C) == (2, 2048, 1024)
        NC = C // 128
        KH = C // 2
        PADF, GAP = 16, 8
        MT = (336, 352)
        T0 = (0, MT[0])
        NT = sum(MT)
        XR = PADF + 6 * NT + 24
        OR = 6 * NT + 16
        B1 = S + GAP

        def kern(x_hbm, w_hbm, m_hbm, v_hbm, g_hbm, b_hbm, o_hbm,
                 xs, osb, of0, of1, wl, wh, acc, pm, pv_, pg, pb, xsem, wsem, osem, psem, *bufs):
            ug = bufs[0:6]; uh = bufs[6:6 + NC]; vs = (bufs[6 + NC:6 + 2 * NC], bufs[6 + 2 * NC:6 + 3 * NC]); va0 = bufs[6 + 3 * NC]
            xs32 = xs.bitcast(U32)
            wh32 = wh.bitcast(U32)
            os32 = osb.bitcast(U32)
            def u_ref(j, i, k):
                if k >= 4: return uh[j], (i - 1,), 4
                if k == 0: return ug[j // 4], (j % 4, i - 1), 0
                if k == 1: return ug[2], (j, i - 1), 1
                if j < 4: return ug[3], (j, i - 1), 2
                return ug[2 + k], (j - 4, i - 1), k
            def u_load(j0, j1, i, k0, k1):
                if i in (0, 7):
                    t = 0 if i == 0 else 2
                    if k0 >= 4: return bf(cat([wh32[j, t] for j in range(j0, j1)], 1))
                    return wl[t, k0 * 128:k1 * 128, j0 * 128:j1 * 128]
                def col(j):
                    pieces = ((0, 1), (1, 2), (2, 4), (4, 8)) if j < 4 else ((0, 1), (1, 2), (2, 3), (3, 4), (4, 8))
                    out = []
                    for (p, e) in pieces:
                        if k0 <= p and e <= k1:
                            buf, idx, _ = u_ref(j, i, p)
                            out.append(buf.bitcast(U32)[idx])
                    return cat(out, 0)
                return bf(cat([col(j) for j in range(j0, j1)], 1))
            def v_load(ch, i, k0, k1, m0=0, m1=None):
                m1 = MT[ch] if m1 is None else m1
                return bf(cat([vs[ch][c].bitcast(U32)[i, m0 // 2:m1 // 2, :] for c in range(k0, k1)], 1))

            def xcopy(bb, c, s):
                return pltpu.make_async_copy(x_hbm.at[bb, :, pl.ds(c * 128, 128)],
                                             xs.at[c, pl.ds(PADF + bb * B1, S), :], xsem.at[s])
            def wcopy(k, s):
                return pltpu.make_async_copy(w_hbm.at[:, pl.ds(k * 128, 128), :], wl.at[:, pl.ds(k * 128, 128), :], wsem.at[s])
            def whis(j0, j1, s):
                return [pltpu.make_async_copy(w_hbm.at[t, pl.ds(KH, KH), pl.ds(j * 128, 128)], wh.at[j, t], wsem.at[s])
                        for j in range(j0, j1) for t in range(3)]
            def wq(t, k, h, s):
                return pltpu.make_async_copy(w_hbm.at[t, pl.ds(k * 128, 128), pl.ds(h * KH, KH)],
                                             wl.at[t, pl.ds(k * 128, 128), pl.ds(h * KH, KH)], wsem.at[s])
            RA = 6 * MA + 16
            def xpart(r0, n, s):
                return pltpu.make_async_copy(x_hbm.at[0, pl.ds(r0, n), pl.ds(0, 128)], xs.at[0, pl.ds(PADF + r0, n), :], xsem.at[s])
            def ocopy1(bb, c, r0, n):
                return pltpu.make_async_copy(osb.at[c, pl.ds(bb * B1 + r0, n), :],
                                             o_hbm.at[bb, pl.ds(r0, n), pl.ds(c * 128, 128)], osem.at[0])
            def ocopies(c, q0, q1):
                out = []
                for bb in range(2):
                    lo_, hi_ = max(q0, bb * B1), min(q1, bb * B1 + S)
                    if hi_ > lo_: out.append(ocopy1(bb, c, lo_ - bb * B1, hi_ - lo_))
                return out
            par = (pm, pv_, pg, pb)
            pcopies = [pltpu.make_async_copy(r, par[i], psem.at[0]) for i, r in enumerate((m_hbm, v_hbm, g_hbm, b_hbm))]
            def start(cs):
                for c in cs: c.start()
            def wait(cs):
                for c in cs: c.wait()
            g_w1 = [wq(t, 0, 0, 4) for t in range(3)]
            g_xa0 = [xpart(0, RA, 0)]
            g_w2 = [wq(t, 0, 1, 5) for t in range(3)] + [xpart(RA, S - RA, 5)]
            g_k1 = [xcopy(0, 1, 1), wcopy(1, 1)]
            g_k23 = [xcopy(0, 2, 2), wcopy(2, 2), xcopy(0, 3, 2)] + [wq(t, 3, 0, 2) for t in range(3)]
            g_x47 = [xcopy(0, c, 3) for c in range(4, 8)] + [wq(t, 3, 1, 3) for t in range(3)]
            g_h1 = whis(0, g1, 3)
            g_h2 = whis(g1, NC, 0)
            g_xa = [xcopy(1, c, 4) for c in range(nxa)]
            g_xb = [xcopy(1, c, 0) for c in range(nxa, 8)]

            def tap_loop(h, s):
                def body(t, carry):
                    wq(t, 0, h, s).start()
                    return carry
                jax.lax.fori_loop(0, 3, body, 0)
            tap_loop(0, 4)
            start(g_xa0)
            zero = jax.lax.fori_loop(0, 8, lambda i, c: c >> 1, 21)
            start(g_w2[3:])
            tap_loop(1, 5)
            start(g_k1)
            for c in range(NC):
                for r0, n in ((0, PADF), (PADF + S, GAP), (PADF + B1 + S, XR - (PADF + B1 + S))):
                    xs[c, pl.ds(r0, n), :] = jnp.zeros((n, 128), BF16)
            views = {}
            def shifted(buf):
                if id(buf) not in views:
                    idx = (slice(None),) * (len(buf.shape) - 2) + (pl.ds(pl.multiple_of(zero, 16), buf.shape[-2]), slice(None))
                    views[id(buf)] = buf.at[idx]
                return views[id(buf)]
            def hold(gv, v, d=0):
                if gv is None: return v
                return jnp.where(jnp.full((8, 128), zero, jnp.int32) == 0, v, pltpu.bitcast(gv(d), v.dtype))

            def w_item(j, r0, gv):
                if r0 >= KH:
                    raw = [wh32[j, k, pl.ds((r0 - KH) // 2, 8), :] for k in range(3)]
                else:
                    raw = [pltpu.bitcast(wl[k, pl.ds(r0, 16), pl.ds(j * 128, 128)], U32) for k in range(3)]
                if wsplit and gv is not None:
                    t = [bf(hold(gv, u)).astype(F32)[0:8] for u in raw]
                    s_ = [bf(hold(gv, u, wsplit)).astype(F32)[8:16] for u in raw]
                    us = [cat(p, 0) for p in zip(gt_(*t), gt_(*s_))]
                else:
                    us = gt_(*(bf(hold(gv, u)).astype(F32) for u in raw))
                for i in range(1, 7):
                    buf, idx, kb = u_ref(j, i, r0 // 128)
                    shifted(buf)[idx + (pl.ds(r0 - 128 * kb, 16), slice(None))] = us[i - 1].astype(BF16)
            def w_items(js, k0, k1):
                return [functools.partial(w_item, j, r0) for j in js for r0 in range(k0 * 128, k1 * 128, 16)]

            def unpackers(gv, d=0):
                mk = hold(gv, jnp.full((8, 128), 0xFFFF0000, U32), d)
                sa = hold(gv, jnp.full((8, 128), 16, U32), d)
                return (lambda u: pltpu.bitcast(u << sa, F32)), (lambda u: pltpu.bitcast(u & mk, F32))
            vfirst = [[] for _ in range(NP)]
            vf16 = {}
            def x_item(ch, c, t0, gv):
                lo, hi = unpackers(gv)
                base = PADF // 2 + 3 * (T0[ch] + t0)
                u = [xs32[c, pl.ds(base + o, 8, stride=6), :] for o in range(-1, 7)]
                e = [hi(u[0])]
                for o in range(1, 4): e += [lo(u[o]), hi(u[o])]
                e.append(lo(u[4]))
                lo, hi = unpackers(gv, dgx)
                e.append(hi(u[4]))
                for o in range(5, 7): e += [lo(u[o]), hi(u[o])]
                e.append(lo(u[7]))
                ve = bt(*e[0:8]); vo = bt(*e[6:14])
                first = ch == 0 and c == 0 and t0 < MA
                for i in range(NP):
                    if first and ssa0:
                        vfirst[i] += [ve[i], vo[i]]
                        continue
                    v = cat([ve[i], vo[i]], 0).astype(BF16)
                    if first: va0[i, pl.ds(t0, 16), :] = v
                    else: shifted(vs[ch][c])[i, pl.ds(t0, 16), :] = v
            def x_items(ch, cs):
                return [functools.partial(x_item, ch, c, t0) for c in cs for t0 in range(0, MT[ch], 16)]

            def place(items, gates, f0, f1):
                for k, it in enumerate(items):
                    gi = min(int(len(gates) * (f0 + (f1 - f0) * k / len(items))), len(gates) - 1)
                    def val(d, gi=gi):
                        arr, r = gates[min(gi + d, len(gates) - 1)]
                        return arr[r:r + 8, 0:128]
                    it(val)

            def dot_a(i, k0, k1, ja=0, jb=NC):
                lhs = v_load(0, i, k0, k1)
                gw = 4 // (k1 - k0)
                gates = []
                for j0 in range(ja, jb, gw):
                    cols = slice(j0 * 128, (j0 + gw) * 128)
                    r = acc[i, 0:MT[0], cols] + mm(lhs, u_load(j0, j0 + gw, i, k0, k1))
                    acc[i, 0:MT[0], cols] = r
                    gates += [(r, rr) for rr in range(0, MT[0], 8)]
                return gates
            def dots_a(idx, k0, k1, ja=0, jb=NC):
                return sum((dot_a(i, k0, k1, ja, jb) for i in idx), [])
            def dot_0(i, part, h):
                m0, m1 = (0, MA) if part == 0 else (MA, MT[0])
                if part == 0 and ssa0:
                    if i not in vf16: vf16[i] = cat(vfirst[i], 0).astype(BF16)
                    lhs = vf16[i]
                else:
                    lhs = va0[i] if part == 0 else v_load(0, i, 0, 1, m0, m1)
                r = mm(lhs, u_load(4 * h, 4 * h + 4, i, 0, 1))
                acc[i, m0:m1, h * KH:(h + 1) * KH] = r
                return [(r, rr) for rr in range(0, m1 - m0, 8)]
            def dots_0(idx, part, h):
                return sum((dot_0(i, part, h) for i in idx), [])

            def epilogue(M, ch, c, m0, m1, send=True):
                sc, sh = bn
                of = (of0, of1)[c % 2]
                scj, shj = sc[:, c * 128:(c + 1) * 128], sh[:, c * 128:(c + 1) * 128]
                ka = [scj] + [(a ** k) * scj for k in range(1, 6)]
                kb = [scj] + [(b ** k) * scj for k in range(1, 6)]
                def silu(h): return h * jnp.tanh(h) + h
                def put(r0, p, h):
                    o = silu(h)
                    for par_ in range(2):
                        of[pl.ds(6 * (m0 + r0 + par_) + p, 8, stride=12), :] = o[8 * par_:8 * par_ + 8]
                def flush(r0):
                    for q in range(6 * (m0 + r0), 6 * (m0 + r0 + 16), 16):
                        osb[c, pl.ds(6 * T0[ch] + q, 16), :] = (shifted(of) if oflag else of)[pl.ds(q, 16), :].astype(BF16)
                def put2(r0, p, lo, hi):
                    if omode == 'rne':
                        l = pltpu.bitcast(lo.astype(BF16).astype(F32), U32) >> 16
                        h = pltpu.bitcast(hi.astype(BF16).astype(F32), U32)
                    else:
                        l = (pltpu.bitcast(lo, U32) + jnp.uint32(0x8000)) >> 16
                        h = (pltpu.bitcast(hi, U32) + jnp.uint32(0x8000)) & jnp.uint32(0xFFFF0000)
                    v = l | h
                    for par_ in range(2):
                        os32[c, pl.ds(3 * (T0[ch] + m0 + r0 + par_) + p, 8, stride=6), :] = v[8 * par_:8 * par_ + 8]
                later = []
                for r0 in range(0, m1 - m0, 16):
                    m = [q[r0:r0 + 16] for q in M]
                    p1 = ((m[1] + m[2]) * scj + shj, (m[1] - m[2]) * scj + shj)
                    pa = (m[3] + m[4], m[3] - m[4]); pb_ = (m[5] + m[6], m[5] - m[6])
                    kk = list(ka)
                    for k in (1, 3, 5):
                        gk = hold(lambda d: m[5][0:8], jnp.broadcast_to(ka[k], (8, 128)))
                        kk[k] = cat([gk, gk], 0)
                    hs = [(p1[k % 2] + pa[k % 2] * kk[k]) + pb_[k % 2] * kb[k] for k in range(6)]
                    hs[0] = hs[0] + m[0] * scj
                    hs[5] = hs[5] + m[7] * scj
                    if omode != 'f32':
                        if defer:
                            for k, gi in ((1, 0), (4, 7)):
                                hs[k] = cat([hold(lambda d: m[gi][e:e + 8], hs[k][e:e + 8]) for e in (0, 8)], 0)
                        o = [silu(h) for h in hs]
                        for p in range(3): put2(r0, p, o[2 * p], o[2 * p + 1])
                        continue
                    for p in range(1, 5): put(r0, p, hs[p])
                    later.append((r0, hs[0], hs[5]))
                for r0, h0, _ in later: put(r0, 0, h0)
                for n_, (r0, _, h5) in enumerate(later):
                    put(r0, 5, h5)
                    if n_ >= lag: flush(later[n_ - lag][0])
                for r0, _, _ in later[max(len(later) - lag, 0):]: flush(r0)
                if send:
                    for cp in ocopies(c, 6 * (T0[ch] + m0), 6 * (T0[ch] + m1)): cp.start(priority=oprio)

            allj = range(NC)
            with scope('w_w1'):
                wait(g_w1)
            with scope('W1'):
                start(g_k23)
                for it in w_items(range(4), 0, 1): it(None)
            with scope('w_xa0'):
                wait(g_xa0)
            x0 = x_items(0, [0])
            with scope('S2'):
                for it in x0[:MA // 16]: it(None)
                dots_0(range(NP), 0, 0)
            with scope('w_w2'):
                wait(g_w2)
            with scope('s0'):
                gt = dots_0((0, 7), 0, 1)
                xb0 = x0[MA // 16:]
                for it in xb0[:3]: it(None)
                place(xb0[3:], gt, tb[0], tb[1])
                gt = gt + dots_0(range(NP), 1, 0)
                place(w_items(range(4, 8), 0, 1), gt, wb[0], wb[1])
                dots_0((0, 7), 1, 1)
                for i in range(1, s0n + 1): dots_0((i,), 0, 1); dots_0((i,), 1, 1)
                start(g_x47); start(pcopies)
            with scope('w_k1'):
                wait(g_k1)
            with scope('s1'):
                gt = []
                for i in range(s0n + 1, 7): gt += dots_0((i,), 0, 1) + dots_0((i,), 1, 1)
                place(x_items(0, [1]), gt, 0.0, s1t)
                gt += dots_a((0, 7), 1, 2)
                place(w_items(allj, 1, 2), gt, s1w[0], s1w[1])
                dots_a(range(1, s1n + 1), 1, 2)
                start(g_h1)
            with scope('w_k23'):
                wait(g_k23)
            with scope('s2'):
                gt = dots_a(range(s1n + 1, 7), 1, 2)
                x2 = x_items(0, [2])
                for it in x2[:t2free]: it(None)
                place(x2[t2free:], gt, 0.0, t2e)
                gt = dots_a((0, 7), 2, 3)
                place(x_items(0, [3]), gt, 0.0, t3e)
                gt = gt + dots_a((0, 7), 3, 4, 0, 4)
                place(w_items(range(4, 8), 2, 3), gt, s2w[0], s2w[1])
                gt = dots_a(range(1, 7), 2, 3, 4, 8)
                place(w_items(range(4), 2, 4), gt, 0.0, 0.9)
                dots_a(range(1, s2n + 1), 2, 4, 0, 4)
                start(g_h2); start(g_xa)
            with scope('w_k47'):
                wait(g_x47); wait(g_h1); wait(pcopies)
            pv = [par[i][...].astype(F32).reshape(1, C) for i in range(4)]
            sc = pv[2] * jax.lax.rsqrt(pv[1] + 1e-5)
            bn = (0.5 * sc, 0.5 * (pv[3] - pv[0] * sc))

            def block_b(ch, j, m0, m1, hooks):
                M = [None] * NP; gt = []
                for n_, i in enumerate(order):
                    if n_ in hooks:
                        hooks[n_](); gt = []
                    q = acc[i, m0:m1, j * 128:(j + 1) * 128] + mm(v_load(ch, i, 4, 8, m0, m1), u_load(j, j + 1, i, 4, 8))
                    M[i] = q
                    if i not in skip: gt += [(q, r) for r in range(0, m1 - m0, 8)]
                return M, gt
            def wait_a():
                with scope('w_xa'):
                    wait(g_xa); wait(g_h2)
            def wait_b():
                with scope('w_xb'):
                    wait(g_xb)
            with scope('s3'):
                gt = dots_a(range(s2n + 1, 7), 2, 4, 0, 4) + dots_a((0, 7), 3, 4, 4, 8)
                start(g_xb)
                place(w_items(range(4, 8), 3, 4), gt, 0.0, 0.8)
                gt = gt + dots_a(range(1, 7), 3, 4, 4, 8)
                place(x_items(0, [4, 5, 6, 7]), gt, 0.0, 0.92)
                place(w_items([0], 4, 8), gt, s3n[0], s3n[1])
                def spread(items, p0, p1):
                    wts = [0.0] * NC
                    for j in range(p0[0], min(p1[0], NC)): wts[j] = 1.0 - (p0[1] / NP if j == p0[0] else 0.0)
                    cum = [sum(wts[:j]) / sum(wts) for j in range(NC + 1)]
                    return [items[int(len(items) * cum[j]):int(len(items) * cum[j + 1])] for j in range(NC)]
                xi = [p + q for p, q in zip(spread(x_items(1, range(nxa)), xa, xb), spread(x_items(1, range(nxa, 4)), xb, (NC, 0)))]
                pending = None
                for j in range(NC):
                    hooks = {}
                    if j == xa[0]: hooks[xa[1]] = wait_a
                    if j == xb[0]: hooks[xb[1]] = wait_b
                    if odelay and j == odelay:
                        for jj in range(odelay):
                            for cp in ocopies(jj, 0, 6 * MT[0]): cp.start(priority=oprio)
                    M, gt = block_b(0, j, 0, MT[0], hooks)
                    if j + 1 < NC: place(w_items([j + 1], 4, 8), gt, pf[0], pf[1])
                    if xi[j]: place(xi[j], gt, pf[0], pf[1])
                    epilogue(M, 0, j, 0, MT[0], send=not (j < odelay))
            with scope('c1a'):
                gt = []
                for j in range(NC):
                    for i in range(NP):
                        q = mm(v_load(1, i, 0, 4), u_load(j, j + 1, i, 0, 4))
                        acc[i, :, j * 128:(j + 1) * 128] = q
                        gt += [(q, r) for r in range(0, MT[1], 8)]
                place(x_items(1, range(4, 8)), gt, 0.05, 0.9)
            with scope('c1b'):
                for j in range(NC):
                    m0 = 0
                    for n in (lastsplit if j == NC - 1 else (MT[1],)):
                        M, _ = block_b(1, j, m0, m0 + n, {})
                        epilogue(M, 1, j, m0, m0 + n)
                        m0 += n
            with scope('w_out'):
                for bb in range(2):
                    for c in range(NC): ocopy1(bb, c, 0, S).wait()

        anyspec = pl.BlockSpec(memory_space=pl.ANY)
        return pl.pallas_call(
            kern,
            in_specs=[anyspec] * 6,
            out_specs=anyspec,
            out_shape=jax.ShapeDtypeStruct(x.shape, x.dtype),
            scratch_shapes=[
                pltpu.VMEM((NC, XR, 128), BF16),
                pltpu.VMEM((NC, OR, 128), BF16),
                pltpu.VMEM((6 * MT[1] + 16, 128), F32), pltpu.VMEM((6 * MT[1] + 16, 128), F32),
                pltpu.VMEM((3, KH, C), BF16),
                pltpu.VMEM((NC, 3, KH, 128), BF16),
                pltpu.VMEM((NP, MT[1], C), F32),
                pltpu.VMEM((C,), BF16), pltpu.VMEM((C,), BF16), pltpu.VMEM((C,), BF16), pltpu.VMEM((C,), BF16),
                pltpu.SemaphoreType.DMA((6,)),
                pltpu.SemaphoreType.DMA((6,)),
                pltpu.SemaphoreType.DMA((1,)),
                pltpu.SemaphoreType.DMA((1,)),
                pltpu.VMEM((NC // 2, 6, 128, 128), BF16), pltpu.VMEM((NC // 2, 6, 128, 128), BF16),
                pltpu.VMEM((NC, 6, 128, 128), BF16), pltpu.VMEM((NC // 2, 6, 256, 128), BF16),
                pltpu.VMEM((NC // 2, 6, 128, 128), BF16), pltpu.VMEM((NC // 2, 6, 128, 128), BF16),
            ] + [pltpu.VMEM((6, KH, 128), BF16)] * NC + [pltpu.VMEM((NP, MT[0], 128), BF16)] * NC
              + [pltpu.VMEM((NP, MT[1], 128), BF16)] * NC + [pltpu.VMEM((NP, MA, 128), BF16)],
            compiler_params=pltpu.CompilerParams(vmem_limit_bytes=110 * 2**20, disable_bounds_checks=True,
                                                 disable_semaphore_checks=True),
        )(x, w, mean, var, g, b_)
    return f


_impl = make(defer=True, skip=(6,))


@jax.jit
def pallas_standalone__batchnorm__prompt_kernel(x, w, mean, var, g, b):
    return _impl(x, w, mean, var, g, b)
```

```python
import contextlib
import functools

import jax
import jax.numpy as jnp
import jax.experimental.pallas as pl
import jax.experimental.pallas.tpu as pltpu

F32, U32, BF16 = jnp.float32, jnp.uint32, jnp.bfloat16

A = 0.5
B = 1.0 / A
A2, B2 = A * A, B * B
C1 = 1.0 / (2.0 * (1.0 - A2) * (1.0 - B2))
CA = 1.0 / (2.0 * A2 * (A2 - 1.0) * (A2 - B2))
CB = 1.0 / (2.0 * B2 * (B2 - 1.0) * (B2 - A2))
NP = 8


def _input_transform(d0, d1, d2, d3, d4, d5, d6, d7):
    d64, d42, d53, d31 = d6 - d4, d4 - d2, d5 - d3, d3 - d1
    v0 = (d0 - d6) + (A2 + 1.0 + B2) * d42
    v7 = (d7 - d1) - (A2 + 1.0 + B2) * d53
    e1 = (d6 + d2) - (A2 + B2) * d4
    o1 = (d5 + d1) - (A2 + B2) * d3
    ea, eb = d64 - B2 * d42, d64 - A2 * d42
    oa, ob = A * d53 - B * d31, B * d53 - A * d31
    return v0, e1 + o1, e1 - o1, ea + oa, ea - oa, eb + ob, eb - ob, v7


def _filter_transform(w0, w1, w2):
    e1, o1 = C1 * (w0 + w2), C1 * w1
    ea, oa = CA * w0 + (CA * A2) * w2, (CA * A) * w1
    eb, ob = CB * w0 + (CB * B2) * w2, (CB * B) * w1
    return e1 + o1, e1 - o1, ea + oa, ea - oa, eb + ob, eb - ob


def _bf(u):
    return pltpu.bitcast(u, BF16)


def _mm(a, b):
    return jnp.dot(a, b, preferred_element_type=F32)


def _cat(parts, axis):
    return parts[0] if len(parts) == 1 else jnp.concatenate(parts, axis=axis)


def make(scopes=False, lastsplit=(176, 96, 48, 32), pf=(0.0, 0.9), s0n=4, s1n=5, s2n=4, g1=2, xa=(1, 1), xb=(4, 1),
         nxa=1, t3e=0.9, s3n=(0.45, 0.9), odelay=5, t2free=7, s2w=(0.4, 0.9), t2e=0.5, dgx=2, dgw=2, s1t=0.6,
         s1w=(0.2, 0.8), MA=192, tb=(0.0, 0.2), wb=(0.2, 0.9)):
    scope = jax.named_scope if scopes else (lambda n: contextlib.nullcontext())
    order = (1, 2, 3, 4, 5, 6, 0, 7)

    @jax.jit
    def f(x, w, mean, var, g, b):
        _, S, C = x.shape
        assert x.shape == (2, 2048, 1024) and w.shape == (3, C, C)
        NC = C // 128
        KH = C // 2
        PADF, GAP = 16, 8
        B1 = S + GAP
        MT = (336, 352)
        T0 = (0, MT[0])
        XR = PADF + 6 * sum(MT) + 24
        OR = 6 * sum(MT) + 16
        RA = 6 * MA + 16

        def kern(x_hbm, w_hbm, m_hbm, v_hbm, g_hbm, b_hbm, o_hbm,
                 xs, osb, wl, wh, acc, pm, pv, pg, pb, xsem, wsem, osem, psem, *bufs):
            ug, uh = bufs[0:6], bufs[6:6 + NC]
            vs = (bufs[6 + NC:6 + 2 * NC], bufs[6 + 2 * NC:6 + 3 * NC])
            xs32, os32, wh32 = xs.bitcast(U32), osb.bitcast(U32), wh.bitcast(U32)

            def xrows(bb, c, r0, n, s):
                return pltpu.make_async_copy(x_hbm.at[bb, pl.ds(r0, n), pl.ds(c * 128, 128)],
                                             xs.at[c, pl.ds(PADF + bb * B1 + r0, n), :], xsem.at[s])

            def xcols(bb, cs, s):
                return [xrows(bb, c, 0, S, s) for c in cs]

            def wrows(k, s):
                return [pltpu.make_async_copy(w_hbm.at[:, pl.ds(k * 128, 128), :], wl.at[:, pl.ds(k * 128, 128), :],
                                              wsem.at[s])]

            def whalf(k, h, s):
                return [pltpu.make_async_copy(w_hbm.at[t, pl.ds(k * 128, 128), pl.ds(h * KH, KH)],
                                              wl.at[t, pl.ds(k * 128, 128), pl.ds(h * KH, KH)], wsem.at[s])
                        for t in range(3)]

            def whigh(js, s):
                return [pltpu.make_async_copy(w_hbm.at[t, pl.ds(KH, KH), pl.ds(j * 128, 128)], wh.at[j, t], wsem.at[s])
                        for j in js for t in range(3)]

            def orows(bb, c, r0, n):
                return pltpu.make_async_copy(osb.at[c, pl.ds(bb * B1 + r0, n), :],
                                             o_hbm.at[bb, pl.ds(r0, n), pl.ds(c * 128, 128)], osem.at[0])

            def send(c, t0, t1):
                for bb in range(2):
                    lo, hi = max(6 * t0, bb * B1), min(6 * t1, bb * B1 + S)
                    if hi > lo:
                        orows(bb, c, lo - bb * B1, hi - lo).start(priority=1)

            def start(cs):
                for cp in cs:
                    cp.start()

            def wait(cs):
                for cp in cs:
                    cp.wait()

            g_w1 = whalf(0, 0, 4)
            g_xa0 = [xrows(0, 0, 0, RA, 0)]
            g_w2 = whalf(0, 1, 5) + [xrows(0, 0, RA, S - RA, 5)]
            g_k1 = xcols(0, [1], 1) + wrows(1, 1)
            g_k23 = xcols(0, [2, 3], 2) + wrows(2, 2) + whalf(3, 0, 2)
            g_x47 = xcols(0, range(4, 8), 3) + whalf(3, 1, 3)
            g_par = [pltpu.make_async_copy(src, dst, psem.at[0])
                     for src, dst in ((m_hbm, pm), (v_hbm, pv), (g_hbm, pg), (b_hbm, pb))]
            g_h1, g_h2 = whigh(range(g1), 3), whigh(range(g1, NC), 0)
            g_xa, g_xb = xcols(1, range(nxa), 4), xcols(1, range(nxa, NC), 0)

            def runtime_zero(seed):
                return jax.lax.fori_loop(0, 6, lambda i, c: c >> 1, seed)

            start(g_w1)
            zero = runtime_zero(21)
            start(g_xa0)
            zero = zero + runtime_zero(19)
            start(g_w2)
            zero = zero + runtime_zero(17)
            start(g_k1)
            for c in range(NC):
                for r0, r1 in ((0, PADF), (PADF + S, PADF + B1), (PADF + B1 + S, XR)):
                    xs[c, pl.ds(r0, r1 - r0), :] = jnp.zeros((r1 - r0, 128), BF16)

            views = {}

            def shifted(buf):
                if id(buf) not in views:
                    rows = pl.ds(pl.multiple_of(zero, 16), buf.shape[-2])
                    views[id(buf)] = buf.at[(slice(None),) * (len(buf.shape) - 2) + (rows, slice(None))]
                return views[id(buf)]

            def hold(v, gate):
                return jnp.where(jnp.full((8, 128), zero, jnp.int32) == 0, v, pltpu.bitcast(gate, v.dtype))

            def place(items, gates, f0, f1):
                for k, item in enumerate(items):
                    gi = int(len(gates) * (f0 + (f1 - f0) * k / len(items)))

                    def gate(d, gi=gi):
                        arr, r = gates[min(gi + d, len(gates) - 1)]
                        return arr[r:r + 8, 0:128]
                    item(gate)

            def free(items):
                for item in items:
                    item(None)

            def u_at(j, i, k):
                if k >= 4:
                    return uh[j], (i - 1,), 4
                if k == 0:
                    return ug[j // 4], (j % 4, i - 1), 0
                if k == 1:
                    return ug[2], (j, i - 1), 1
                if j < 4:
                    return ug[3], (j, i - 1), 2
                return ug[2 + k], (j - 4, i - 1), k

            def w_item(j, r0, gate):
                if r0 >= KH:
                    raw = [wh32[j, t, pl.ds((r0 - KH) // 2, 8), :] for t in range(3)]
                else:
                    raw = [pltpu.bitcast(wl[t, pl.ds(r0, 16), pl.ds(j * 128, 128)], U32) for t in range(3)]
                if gate is None:
                    us = _filter_transform(*(_bf(u).astype(F32) for u in raw))
                else:
                    top = _filter_transform(*(_bf(hold(u, gate(0))).astype(F32)[0:8] for u in raw))
                    bot = _filter_transform(*(_bf(hold(u, gate(dgw))).astype(F32)[8:16] for u in raw))
                    us = [_cat(p, 0) for p in zip(top, bot)]
                for i in range(1, 7):
                    buf, idx, kb = u_at(j, i, r0 // 128)
                    shifted(buf)[idx + (pl.ds(r0 - 128 * kb, 16), slice(None))] = us[i - 1].astype(BF16)

            def w_items(js, k0, k1):
                return [functools.partial(w_item, j, r0) for j in js for r0 in range(k0 * 128, k1 * 128, 16)]

            def unpackers(gate, d):
                mask, shift = jnp.full((8, 128), 0xFFFF0000, U32), jnp.full((8, 128), 16, U32)
                if gate is not None:
                    mask, shift = hold(mask, gate(d)), hold(shift, gate(d))
                return (lambda u: pltpu.bitcast(u << shift, F32)), (lambda u: pltpu.bitcast(u & mask, F32))

            v_first = [[] for _ in range(NP)]

            def x_item(ch, c, t0, gate):
                base = PADF // 2 + 3 * (T0[ch] + t0)
                u = [xs32[c, pl.ds(base + o, 8, stride=6), :] for o in range(-1, 7)]
                lo, hi = unpackers(gate, 0)
                d = [hi(u[0]), lo(u[1]), hi(u[1]), lo(u[2]), hi(u[2]), lo(u[3]), hi(u[3]), lo(u[4])]
                lo, hi = unpackers(gate, dgx)
                d += [hi(u[4]), lo(u[5]), hi(u[5]), lo(u[6]), hi(u[6]), lo(u[7])]
                even, odd = _input_transform(*d[0:8]), _input_transform(*d[6:14])
                for i in range(NP):
                    if ch == 0 and c == 0 and t0 < MA:
                        v_first[i] += [even[i], odd[i]]
                    else:
                        shifted(vs[ch][c])[i, pl.ds(t0, 16), :] = _cat([even[i], odd[i]], 0).astype(BF16)

            def x_items(ch, cs):
                return [functools.partial(x_item, ch, c, t0) for c in cs for t0 in range(0, MT[ch], 16)]

            def epilogue(M, ch, c, m0, m1):
                sc, sh = (p[:, c * 128:(c + 1) * 128] for p in bn)
                ka, kb = [A ** k * sc for k in range(6)], [B ** k * sc for k in range(6)]
                for r0 in range(0, m1 - m0, 16):
                    m = [q[r0:r0 + 16] for q in M]
                    p1 = ((m[1] + m[2]) * sc + sh, (m[1] - m[2]) * sc + sh)
                    pa, pb_ = (m[3] + m[4], m[3] - m[4]), (m[5] + m[6], m[5] - m[6])
                    kk = [_cat([hold(jnp.broadcast_to(ka[k], (8, 128)), m[5][0:8])] * 2, 0) if k % 2 else ka[k]
                          for k in range(6)]
                    h = [(p1[k % 2] + pa[k % 2] * kk[k]) + pb_[k % 2] * kb[k] for k in range(6)]
                    h[0] = h[0] + m[0] * sc
                    h[5] = h[5] + m[7] * sc
                    for k, i in ((1, 0), (4, 7)):
                        h[k] = _cat([hold(h[k][e:e + 8], m[i][e:e + 8]) for e in (0, 8)], 0)
                    o = [pltpu.bitcast(q * jnp.tanh(q) + q, U32) + jnp.uint32(0x8000) for q in h]
                    for p in range(3):
                        words = (o[2 * p] >> 16) | (o[2 * p + 1] & jnp.uint32(0xFFFF0000))
                        for par in range(2):
                            row = 3 * (T0[ch] + m0 + r0 + par) + p
                            os32[c, pl.ds(row, 8, stride=6), :] = words[8 * par:8 * par + 8]

            def u_load(i, k0, k1, j0, j1):
                if i in (0, 7):
                    t = 0 if i == 0 else 2
                    if k0 >= 4:
                        return _bf(_cat([wh32[j, t] for j in range(j0, j1)], 1))
                    return wl[t, k0 * 128:k1 * 128, j0 * 128:j1 * 128]

                def col(j):
                    ks = [k for k in range(k0, k1) if u_at(j, i, k)[2] == k]
                    return _cat([u_at(j, i, k)[0].bitcast(U32)[u_at(j, i, k)[1]] for k in ks], 0)
                return _bf(_cat([col(j) for j in range(j0, j1)], 1))

            def v_load(ch, i, k0, k1, m0, m1):
                return _bf(_cat([vs[ch][c].bitcast(U32)[i, m0 // 2:m1 // 2, :] for c in range(k0, k1)], 1))

            def rows8(r):
                return [(r, rr) for rr in range(0, r.shape[0], 8)]

            v0_bf16 = {}

            def dots_0(idx, part, h):
                m0, m1 = (0, MA) if part == 0 else (MA, MT[0])
                gates = []
                for i in idx:
                    if part == 0 and i not in v0_bf16:
                        v0_bf16[i] = _cat(v_first[i], 0).astype(BF16)
                    lhs = v0_bf16[i] if part == 0 else v_load(0, i, 0, 1, m0, m1)
                    r = _mm(lhs, u_load(i, 0, 1, 4 * h, 4 * h + 4))
                    acc[i, m0:m1, h * KH:(h + 1) * KH] = r
                    gates += rows8(r)
                return gates

            def dots_a(idx, k0, k1, j0=0, j1=NC):
                gw = 4 // (k1 - k0)
                gates = []
                for i in idx:
                    lhs = v_load(0, i, k0, k1, 0, MT[0])
                    for j in range(j0, j1, gw):
                        cols = slice(j * 128, (j + gw) * 128)
                        r = acc[i, 0:MT[0], cols] + _mm(lhs, u_load(i, k0, k1, j, j + gw))
                        acc[i, 0:MT[0], cols] = r
                        gates += rows8(r)
                return gates

            def block(ch, j, m0, m1, waits=None):
                M, gates = [None] * NP, []
                for n, i in enumerate(order):
                    if waits is not None and n == waits[0]:
                        with scope('w_x1'):
                            wait(waits[1])
                        gates = []
                    M[i] = acc[i, m0:m1, j * 128:(j + 1) * 128] + _mm(v_load(ch, i, 4, 8, m0, m1), u_load(i, 4, 8, j, j + 1))
                    if i != 6:
                        gates += rows8(M[i])
                return M, gates

            lo_j, hi_j = range(4), range(4, NC)
            with scope('w_w1'):
                wait(g_w1)
            with scope('W1'):
                start(g_k23)
                free(w_items(lo_j, 0, 1))
            with scope('w_xa0'):
                wait(g_xa0)
            x0 = x_items(0, [0])
            with scope('S2'):
                free(x0[:MA // 16])
                dots_0(range(NP), 0, 0)
            with scope('w_w2'):
                wait(g_w2)
            with scope('s0'):
                gt = dots_0((0, 7), 0, 1)
                free(x0[MA // 16:MA // 16 + 3])
                place(x0[MA // 16 + 3:], gt, *tb)
                gt += dots_0(range(NP), 1, 0)
                place(w_items(hi_j, 0, 1), gt, *wb)
                dots_0((0, 7), 1, 1)
                for i in range(1, s0n + 1):
                    dots_0((i,), 0, 1), dots_0((i,), 1, 1)
                start(g_x47 + g_par)
            with scope('w_k1'):
                wait(g_k1)
            with scope('s1'):
                gt = []
                for i in range(s0n + 1, 7):
                    gt += dots_0((i,), 0, 1) + dots_0((i,), 1, 1)
                place(x_items(0, [1]), gt, 0.0, s1t)
                gt += dots_a((0, 7), 1, 2)
                place(w_items(range(NC), 1, 2), gt, *s1w)
                dots_a(range(1, s1n + 1), 1, 2)
                start(g_h1)
            with scope('w_k23'):
                wait(g_k23)
            with scope('s2'):
                gt = dots_a(range(s1n + 1, 7), 1, 2)
                x2 = x_items(0, [2])
                free(x2[:t2free])
                place(x2[t2free:], gt, 0.0, t2e)
                gt = dots_a((0, 7), 2, 3)
                place(x_items(0, [3]), gt, 0.0, t3e)
                gt += dots_a((0, 7), 3, 4, 0, 4)
                place(w_items(hi_j, 2, 3), gt, *s2w)
                gt = dots_a(range(1, 7), 2, 3, 4, NC)
                place(w_items(lo_j, 2, 4), gt, 0.0, 0.9)
                dots_a(range(1, s2n + 1), 2, 4, 0, 4)
                start(g_h2 + g_xa)
            with scope('w_k47'):
                wait(g_x47 + g_h1 + g_par)
            mean_, var_, g_, b_ = (p[...].astype(F32).reshape(1, C) for p in (pm, pv, pg, pb))
            scale = g_ * jax.lax.rsqrt(var_ + 1e-5)
            bn = (0.5 * scale, 0.5 * (b_ - mean_ * scale))
            with scope('s3'):
                gt = dots_a(range(s2n + 1, 7), 2, 4, 0, 4) + dots_a((0, 7), 3, 4, 4, NC)
                start(g_xb)
                place(w_items(hi_j, 3, 4), gt, 0.0, 0.8)
                gt += dots_a(range(1, 7), 3, 4, 4, NC)
                place(x_items(0, range(4, NC)), gt, 0.0, 0.92)
                place(w_items([0], 4, 8), gt, *s3n)

                def spread(items, j0, j1):
                    wts = [(1.0 - j0[1] / NP if j == j0[0] else 1.0) if j0[0] <= j < j1 else 0.0 for j in range(NC)]
                    cum = [int(len(items) * sum(wts[:j]) / sum(wts)) for j in range(NC + 1)]
                    return [items[cum[j]:cum[j + 1]] for j in range(NC)]
                x1 = [p + q for p, q in zip(spread(x_items(1, range(nxa)), xa, xb[0]),
                                            spread(x_items(1, range(nxa, 4)), xb, NC))]
                for j in range(NC):
                    if j == odelay:
                        for jj in range(odelay):
                            send(jj, 0, MT[0])
                    waits = {xa[0]: (xa[1], g_xa + g_h2), xb[0]: (xb[1], g_xb)}.get(j)
                    M, gt = block(0, j, 0, MT[0], waits)
                    if j + 1 < NC:
                        place(w_items([j + 1], 4, 8), gt, *pf)
                    if x1[j]:
                        place(x1[j], gt, *pf)
                    epilogue(M, 0, j, 0, MT[0])
                    if j >= odelay:
                        send(j, 0, MT[0])

            with scope('c1a'):
                gt = []
                for j in range(NC):
                    for i in range(NP):
                        r = _mm(v_load(1, i, 0, 4, 0, MT[1]), u_load(i, 0, 4, j, j + 1))
                        acc[i, :, j * 128:(j + 1) * 128] = r
                        gt += rows8(r)
                place(x_items(1, range(4, NC)), gt, 0.05, 0.9)
            with scope('c1b'):
                for j in range(NC):
                    m0 = 0
                    for n in (lastsplit if j == NC - 1 else (MT[1],)):
                        M, _ = block(1, j, m0, m0 + n)
                        epilogue(M, 1, j, m0, m0 + n)
                        send(j, T0[1] + m0, T0[1] + m0 + n)
                        m0 += n
            with scope('w_out'):
                wait([orows(bb, c, 0, S) for bb in range(2) for c in range(NC)])

        vmem = pltpu.VMEM
        return pl.pallas_call(
            kern,
            in_specs=[pl.BlockSpec(memory_space=pl.ANY)] * 6,
            out_specs=pl.BlockSpec(memory_space=pl.ANY),
            out_shape=jax.ShapeDtypeStruct(x.shape, x.dtype),
            scratch_shapes=[
                vmem((NC, XR, 128), BF16), vmem((NC, OR, 128), BF16),
                vmem((3, KH, C), BF16), vmem((NC, 3, KH, 128), BF16),
                vmem((NP, MT[1], C), F32),
                vmem((C,), BF16), vmem((C,), BF16), vmem((C,), BF16), vmem((C,), BF16),
                pltpu.SemaphoreType.DMA((6,)), pltpu.SemaphoreType.DMA((6,)),
                pltpu.SemaphoreType.DMA((1,)), pltpu.SemaphoreType.DMA((1,)),
                vmem((4, 6, 128, 128), BF16), vmem((4, 6, 128, 128), BF16), vmem((NC, 6, 128, 128), BF16),
                vmem((4, 6, 256, 128), BF16), vmem((4, 6, 128, 128), BF16), vmem((4, 6, 128, 128), BF16),
            ] + [vmem((6, KH, 128), BF16)] * NC + [vmem((NP, MT[0], 128), BF16)] * NC + [vmem((NP, MT[1], 128), BF16)] * NC,
            compiler_params=pltpu.CompilerParams(vmem_limit_bytes=110 * 2 ** 20, disable_bounds_checks=True,
                                                 disable_semaphore_checks=True),
        )(x, w, mean, var, g, b)
    return f


pallas_standalone__batchnorm__prompt_kernel = make()
```

```python
import contextlib
import functools

import jax
import jax.numpy as jnp
import jax.experimental.pallas as pl
import jax.experimental.pallas.tpu as pltpu

F32, U32, BF16 = jnp.float32, jnp.uint32, jnp.bfloat16

A = 0.5
B = 1.0 / A
A2, B2 = A * A, B * B
C1 = 1.0 / (2.0 * (1.0 - A2) * (1.0 - B2))
CA = 1.0 / (2.0 * A2 * (A2 - 1.0) * (A2 - B2))
CB = 1.0 / (2.0 * B2 * (B2 - 1.0) * (B2 - A2))
NP = 8


def _input_transform(d0, d1, d2, d3, d4, d5, d6, d7):
    d64, d42, d53, d31 = d6 - d4, d4 - d2, d5 - d3, d3 - d1
    v0 = (d0 - d6) + (A2 + 1.0 + B2) * d42
    v7 = (d7 - d1) - (A2 + 1.0 + B2) * d53
    e1 = (d6 + d2) - (A2 + B2) * d4
    o1 = (d5 + d1) - (A2 + B2) * d3
    ea, eb = d64 - B2 * d42, d64 - A2 * d42
    oa, ob = A * d53 - B * d31, B * d53 - A * d31
    return v0, e1 + o1, e1 - o1, ea + oa, ea - oa, eb + ob, eb - ob, v7


def _filter_transform(w0, w1, w2):
    e1, o1 = C1 * (w0 + w2), C1 * w1
    ea, oa = CA * w0 + (CA * A2) * w2, (CA * A) * w1
    eb, ob = CB * w0 + (CB * B2) * w2, (CB * B) * w1
    return e1 + o1, e1 - o1, ea + oa, ea - oa, eb + ob, eb - ob


def _bf(u):
    return pltpu.bitcast(u, BF16)


def _mm(a, b):
    return jnp.dot(a, b, preferred_element_type=F32)


def _cat(parts, axis):
    return parts[0] if len(parts) == 1 else jnp.concatenate(parts, axis=axis)


def make(scopes=False, lastsplit=(176, 96, 48, 32), pf=(0.0, 1.0), s0n=4, s1n=5, s2n=2, nf=33, merged=False, cf=(0.0, 0.95), gset=(1, 2, 3),
         t3e=0.9, t2free=7, s2w=(0.4, 0.9), t2e=0.5, dgx=2, dgw=2, s1t=0.6,
         s1w=(0.2, 0.8), MA=192, tb=(0.0, 0.2), wb=(0.2, 0.9)):
    scope = jax.named_scope if scopes else (lambda n: contextlib.nullcontext())
    order = (1, 2, 3, 4, 5, 6, 0, 7)

    @jax.jit
    def f(x, w, mean, var, g, b):
        _, S, C = x.shape
        assert x.shape == (2, 2048, 1024) and w.shape == (3, C, C)
        NC = C // 128
        KH = C // 2
        PADF, GAP = 16, 8
        B1 = S + GAP
        MT = (336, 352)
        T0 = (0, MT[0])
        NT = sum(MT)
        XR = PADF + 6 * NT + 24
        OR = 6 * NT + 16
        RA = 6 * MA + 16

        def kern(x_hbm, w_hbm, m_hbm, v_hbm, g_hbm, b_hbm, o_hbm,
                 xs, osb, wl, wh, acc, pm, pv, pg, pb, xsem, wsem, osem, psem, *bufs):
            ug, uh = bufs[0:6], bufs[6:6 + NC]
            vs = (bufs[6 + NC:6 + 2 * NC], bufs[6 + 2 * NC:6 + 3 * NC])
            xs32, os32, wh32 = xs.bitcast(U32), osb.bitcast(U32), wh.bitcast(U32)

            def xrows(bb, c, r0, n, s):
                return pltpu.make_async_copy(x_hbm.at[bb, pl.ds(r0, n), pl.ds(c * 128, 128)],
                                             xs.at[c, pl.ds(PADF + bb * B1 + r0, n), :], xsem.at[s])

            def xcols(bb, cs, s):
                return [xrows(bb, c, 0, S, s) for c in cs]

            def wrows(k, s):
                return [pltpu.make_async_copy(w_hbm.at[:, pl.ds(k * 128, 128), :], wl.at[:, pl.ds(k * 128, 128), :],
                                              wsem.at[s])]

            def whalf(k, h, s):
                return [pltpu.make_async_copy(w_hbm.at[t, pl.ds(k * 128, 128), pl.ds(h * KH, KH)],
                                              wl.at[t, pl.ds(k * 128, 128), pl.ds(h * KH, KH)], wsem.at[s])
                        for t in range(3)]

            def whigh(js, s):
                return [pltpu.make_async_copy(w_hbm.at[t, pl.ds(KH, KH), pl.ds(j * 128, 128)], wh.at[j, t], wsem.at[s])
                        for j in js for t in range(3)]

            def orows(bb, c, r0, n):
                return pltpu.make_async_copy(osb.at[c, pl.ds(bb * B1 + r0, n), :],
                                             o_hbm.at[bb, pl.ds(r0, n), pl.ds(c * 128, 128)], osem.at[0])

            def send(c, t0, t1):
                for bb in range(2):
                    lo, hi = max(6 * t0, bb * B1), min(6 * t1, bb * B1 + S)
                    if hi > lo:
                        orows(bb, c, lo - bb * B1, hi - lo).start(priority=1)

            def start(cs):
                for cp in cs:
                    cp.start()

            def wait(cs):
                for cp in cs:
                    cp.wait()

            g_w1 = whalf(0, 0, 4)
            g_xa0 = [xrows(0, 0, 0, RA, 0)]
            g_w2 = whalf(0, 1, 5) + [xrows(0, 0, RA, S - RA, 5)]
            g_k1 = xcols(0, [1], 1) + wrows(1, 1)
            g_k23 = xcols(0, [2, 3], 2) + wrows(2, 2) + whalf(3, 0, 2)
            g_x1 = xcols(1, range(4), 3) + whalf(3, 1, 3)
            g_par = [pltpu.make_async_copy(src, dst, psem.at[0])
                     for src, dst in ((m_hbm, pm), (v_hbm, pv), (g_hbm, pg), (b_hbm, pb))]
            g_rest = xcols(0, range(4, NC), 4) + xcols(1, range(4, NC), 4) + whigh(range(NC), 0) + g_par

            def runtime_zero(seed):
                return jax.lax.fori_loop(0, 6, lambda i, c: c >> 1, seed)

            start(g_w1)
            zero = runtime_zero(21)
            start(g_xa0)
            zero = zero + runtime_zero(19)
            start(g_w2)
            zero = zero + runtime_zero(17)
            start(g_k1)
            for c in range(NC):
                for r0, r1 in ((0, PADF), (PADF + S, PADF + B1), (PADF + B1 + S, XR)):
                    xs[c, pl.ds(r0, r1 - r0), :] = jnp.zeros((r1 - r0, 128), BF16)

            views = {}

            def shifted(buf):
                if id(buf) not in views:
                    rows = pl.ds(pl.multiple_of(zero, 16), buf.shape[-2])
                    views[id(buf)] = buf.at[(slice(None),) * (len(buf.shape) - 2) + (rows, slice(None))]
                return views[id(buf)]

            def hold(v, gate):
                return jnp.where(jnp.full((8, 128), zero, jnp.int32) == 0, v, pltpu.bitcast(gate, v.dtype))

            def place(items, gates, f0, f1):
                for k, item in enumerate(items):
                    gi = int(len(gates) * (f0 + (f1 - f0) * k / len(items)))

                    def gate(d, gi=gi):
                        arr, r = gates[min(gi + d, len(gates) - 1)]
                        return arr[r:r + 8, 0:128]
                    item(gate)

            def free(items):
                for item in items:
                    item(None)

            def u_at(j, i, k):
                if k >= 4:
                    return uh[j], (i - 1,), 4
                if k == 0:
                    return ug[j // 4], (j % 4, i - 1), 0
                if k == 1:
                    return ug[2], (j, i - 1), 1
                if j < 4:
                    return ug[3], (j, i - 1), 2
                return ug[2 + k], (j - 4, i - 1), k

            def w_item(j, r0, gate):
                if r0 >= KH:
                    raw = [wh32[j, t, pl.ds((r0 - KH) // 2, 8), :] for t in range(3)]
                else:
                    raw = [pltpu.bitcast(wl[t, pl.ds(r0, 16), pl.ds(j * 128, 128)], U32) for t in range(3)]
                if gate is None:
                    us = _filter_transform(*(_bf(u).astype(F32) for u in raw))
                else:
                    top = _filter_transform(*(_bf(hold(u, gate(0))).astype(F32)[0:8] for u in raw))
                    bot = _filter_transform(*(_bf(hold(u, gate(dgw))).astype(F32)[8:16] for u in raw))
                    us = [_cat(p, 0) for p in zip(top, bot)]
                for i in range(1, 7):
                    buf, idx, kb = u_at(j, i, r0 // 128)
                    shifted(buf)[idx + (pl.ds(r0 - 128 * kb, 16), slice(None))] = us[i - 1].astype(BF16)

            def w_items(js, k0, k1):
                return [functools.partial(w_item, j, r0) for j in js for r0 in range(k0 * 128, k1 * 128, 16)]

            def unpackers(gate, d):
                mask, shift = jnp.full((8, 128), 0xFFFF0000, U32), jnp.full((8, 128), 16, U32)
                if gate is not None:
                    mask, shift = hold(mask, gate(d)), hold(shift, gate(d))
                return (lambda u: pltpu.bitcast(u << shift, F32)), (lambda u: pltpu.bitcast(u & mask, F32))

            v_first = [[] for _ in range(NP)]

            def x_item(ch, c, t0, gate):
                base = PADF // 2 + 3 * (T0[ch] + t0)
                u = [xs32[c, pl.ds(base + o, 8, stride=6), :] for o in range(-1, 7)]
                lo, hi = unpackers(gate, 0)
                d = [hi(u[0]), lo(u[1]), hi(u[1]), lo(u[2]), hi(u[2]), lo(u[3]), hi(u[3]), lo(u[4])]
                lo, hi = unpackers(gate, dgx)
                d += [hi(u[4]), lo(u[5]), hi(u[5]), lo(u[6]), hi(u[6]), lo(u[7])]
                even, odd = _input_transform(*d[0:8]), _input_transform(*d[6:14])
                for i in range(NP):
                    if ch == 0 and c == 0 and t0 < MA:
                        v_first[i] += [even[i], odd[i]]
                    else:
                        shifted(vs[ch][c])[i, pl.ds(t0, 16), :] = _cat([even[i], odd[i]], 0).astype(BF16)

            def x_items(ch, cs):
                return [functools.partial(x_item, ch, c, t0) for c in cs for t0 in range(0, MT[ch], 16)]

            def epilogue(M, c, m0, m1):
                sc, sh = (p[:, c * 128:(c + 1) * 128] for p in bn)
                ka, kb = [A ** k * sc for k in range(6)], [B ** k * sc for k in range(6)]
                for r0 in range(0, m1 - m0, 16):
                    m = [q[r0:r0 + 16] for q in M]
                    p1 = ((m[1] + m[2]) * sc + sh, (m[1] - m[2]) * sc + sh)
                    pa, pb_ = (m[3] + m[4], m[3] - m[4]), (m[5] + m[6], m[5] - m[6])
                    kk = [_cat([hold(jnp.broadcast_to(ka[k], (8, 128)), m[5][0:8])] * 2, 0) if k % 2 else ka[k]
                          for k in range(6)]
                    h = [(p1[k % 2] + pa[k % 2] * kk[k]) + pb_[k % 2] * kb[k] for k in range(6)]
                    h[0] = h[0] + m[0] * sc
                    h[5] = h[5] + m[7] * sc
                    for k, i in ((1, 0), (4, 7)):
                        h[k] = _cat([hold(h[k][e:e + 8], m[i][e:e + 8]) for e in (0, 8)], 0)
                    o = [pltpu.bitcast(q * jnp.tanh(q) + q, U32) + jnp.uint32(0x8000) for q in h]
                    for p in range(3):
                        words = (o[2 * p] >> 16) | (o[2 * p + 1] & jnp.uint32(0xFFFF0000))
                        for par in range(2):
                            row = 3 * (m0 + r0 + par) + p
                            os32[c, pl.ds(row, 8, stride=6), :] = words[8 * par:8 * par + 8]

            def u_load(i, k0, k1, j0, j1):
                if i in (0, 7):
                    t = 0 if i == 0 else 2
                    if k0 >= 4:
                        return _bf(_cat([wh32[j, t] for j in range(j0, j1)], 1))
                    return wl[t, k0 * 128:k1 * 128, j0 * 128:j1 * 128]

                def col(j):
                    ks = [k for k in range(k0, k1) if u_at(j, i, k)[2] == k]
                    return _cat([u_at(j, i, k)[0].bitcast(U32)[u_at(j, i, k)[1]] for k in ks], 0)
                return _bf(_cat([col(j) for j in range(j0, j1)], 1))

            def v_load(ch, i, k0, k1, m0, m1):
                return _bf(_cat([vs[ch][c].bitcast(U32)[i, m0 // 2:m1 // 2, :] for c in range(k0, k1)], 1))

            def rows8(r):
                return [(r, rr) for rr in range(0, r.shape[0], 8)]

            v0_bf16 = {}

            def dots_0(idx, part, h):
                m0, m1 = (0, MA) if part == 0 else (MA, MT[0])
                gates = []
                for i in idx:
                    if part == 0 and i not in v0_bf16:
                        v0_bf16[i] = _cat(v_first[i], 0).astype(BF16)
                    lhs = v0_bf16[i] if part == 0 else v_load(0, i, 0, 1, m0, m1)
                    r = _mm(lhs, u_load(i, 0, 1, 4 * h, 4 * h + 4))
                    acc[i, m0:m1, h * KH:(h + 1) * KH] = r
                    gates += rows8(r)
                return gates

            def dots_a(idx, k0, k1, j0=0, j1=NC):
                gw = 4 // (k1 - k0)
                gates = []
                for i in idx:
                    lhs = v_load(0, i, k0, k1, 0, MT[0])
                    for j in range(j0, j1, gw):
                        cols = slice(j * 128, (j + gw) * 128)
                        r = acc[i, 0:MT[0], cols] + _mm(lhs, u_load(i, k0, k1, j, j + gw))
                        acc[i, 0:MT[0], cols] = r
                        gates += rows8(r)
                return gates

            def block(j, t0, t1):
                M, gates = [None] * NP, []
                for i in order:
                    lhs = _cat([v_load(ch, i, 4, NC, max(t0, T0[ch]) - T0[ch], min(t1, T0[ch] + MT[ch]) - T0[ch])
                                for ch in range(2) if max(t0, T0[ch]) < min(t1, T0[ch] + MT[ch])], 0)
                    M[i] = acc[i, t0:t1, j * 128:(j + 1) * 128] + _mm(lhs, u_load(i, 4, NC, j, j + 1))
                    if i in gset:
                        gates += rows8(M[i])
                return M, gates

            lo_j, hi_j = range(4), range(4, NC)
            with scope('w_w1'):
                wait(g_w1)
            with scope('W1'):
                start(g_k23)
                free(w_items(lo_j, 0, 1))
            with scope('w_xa0'):
                wait(g_xa0)
            x0 = x_items(0, [0])
            with scope('S2'):
                free(x0[:MA // 16])
                dots_0(range(NP), 0, 0)
            with scope('w_w2'):
                wait(g_w2)
            with scope('s0'):
                gt = dots_0((0, 7), 0, 1)
                free(x0[MA // 16:MA // 16 + 3])
                place(x0[MA // 16 + 3:], gt, *tb)
                gt += dots_0(range(NP), 1, 0)
                place(w_items(hi_j, 0, 1), gt, *wb)
                dots_0((0, 7), 1, 1)
                for i in range(1, s0n + 1):
                    dots_0((i,), 0, 1), dots_0((i,), 1, 1)
                start(g_x1)
            with scope('w_k1'):
                wait(g_k1)
            with scope('s1'):
                gt = []
                for i in range(s0n + 1, 7):
                    gt += dots_0((i,), 0, 1) + dots_0((i,), 1, 1)
                place(x_items(0, [1]), gt, 0.0, s1t)
                gt += dots_a((0, 7), 1, 2)
                place(w_items(range(NC), 1, 2), gt, *s1w)
                dots_a(range(1, s1n + 1), 1, 2)
            with scope('w_k23'):
                wait(g_k23)
            with scope('s2'):
                gt = dots_a(range(s1n + 1, 7), 1, 2)
                x2 = x_items(0, [2])
                free(x2[:t2free])
                place(x2[t2free:], gt, 0.0, t2e)
                gt = dots_a((0, 7), 2, 3)
                place(x_items(0, [3]), gt, 0.0, t3e)
                gt += dots_a((0, 7), 3, 4, 0, 4)
                place(w_items(hi_j, 2, 3), gt, *s2w)
                gt = dots_a(range(1, 7), 2, 3, 4, NC)
                place(w_items(lo_j, 2, 4), gt, 0.0, 0.9)
                dots_a(range(1, s2n + 1), 2, 4, 0, 4)
                start(g_rest)
            with scope('w_x1'):
                wait(g_x1)
            with scope('s3'):
                gt = dots_a(range(s2n + 1, 7), 2, 4, 0, 4) + dots_a((0, 7), 3, 4, 4, NC)
                place(w_items(hi_j, 3, 4), gt, 0.0, 0.8)
                gt += dots_a(range(1, 7), 3, 4, 4, NC)
                place(x_items(1, range(4)), gt, 0.0, 0.92)

                gt = []
                for n in range(NC * NP):
                    if n == nf:
                        with scope('w_rest'):
                            wait(g_rest)
                        gt = []
                    j, i = divmod(n, NP)
                    r = _mm(v_load(1, i, 0, 4, 0, MT[1]), u_load(i, 0, 4, j, j + 1))
                    acc[i, MT[0]:NT, j * 128:(j + 1) * 128] = r
                    gt += rows8(r)
                mean_, var_, g_, b_ = (p[...].astype(F32).reshape(1, C) for p in (pm, pv, pg, pb))
                scale = g_ * jax.lax.rsqrt(var_ + 1e-5)
                bn = (0.5 * scale, 0.5 * (b_ - mean_ * scale))
                place(x_items(0, range(4, NC)) + x_items(1, range(4, NC)), gt, *cf)
                place(w_items([0], 4, NC), gt, *cf)

            with scope('B'):
                for j in range(NC):
                    cuts = [0] + ([] if merged else [MT[0]])
                    if j == NC - 1:
                        cuts += [NT - sum(lastsplit[k:]) for k in range(len(lastsplit)) if NT - sum(lastsplit[k:]) > cuts[-1]]
                    gt = []
                    for t0, t1 in zip(cuts, cuts[1:] + [NT]):
                        M, gates = block(j, t0, t1)
                        gt += gates
                        epilogue(M, j, t0, t1)
                        send(j, t0, t1)
                    if j + 1 < NC:
                        place(w_items([j + 1], 4, NC), gt, *pf)
            with scope('w_out'):
                wait([orows(bb, c, 0, S) for bb in range(2) for c in range(NC)])

        vmem = pltpu.VMEM
        return pl.pallas_call(
            kern,
            in_specs=[pl.BlockSpec(memory_space=pl.ANY)] * 6,
            out_specs=pl.BlockSpec(memory_space=pl.ANY),
            out_shape=jax.ShapeDtypeStruct(x.shape, x.dtype),
            scratch_shapes=[
                vmem((NC, XR, 128), BF16), vmem((NC, OR, 128), BF16),
                vmem((3, KH, C), BF16), vmem((NC, 3, KH, 128), BF16),
                vmem((NP, NT, C), F32),
                vmem((C,), BF16), vmem((C,), BF16), vmem((C,), BF16), vmem((C,), BF16),
                pltpu.SemaphoreType.DMA((6,)), pltpu.SemaphoreType.DMA((6,)),
                pltpu.SemaphoreType.DMA((1,)), pltpu.SemaphoreType.DMA((1,)),
                vmem((4, 6, 128, 128), BF16), vmem((4, 6, 128, 128), BF16), vmem((NC, 6, 128, 128), BF16),
                vmem((4, 6, 256, 128), BF16), vmem((4, 6, 128, 128), BF16), vmem((4, 6, 128, 128), BF16),
            ] + [vmem((6, KH, 128), BF16)] * NC + [vmem((NP, MT[0], 128), BF16)] * NC + [vmem((NP, MT[1], 128), BF16)] * NC,
            compiler_params=pltpu.CompilerParams(vmem_limit_bytes=110 * 2 ** 20, disable_bounds_checks=True,
                                                 disable_semaphore_checks=True),
        )(x, w, mean, var, g, b)
    return f


pallas_standalone__batchnorm__prompt_kernel = make()
```

```python
import contextlib
import functools

import jax
import jax.numpy as jnp
import jax.experimental.pallas as pl
import jax.experimental.pallas.tpu as pltpu

F32, U32, BF16 = jnp.float32, jnp.uint32, jnp.bfloat16

A = 0.52
B = 1.0 / A
A2, B2 = A * A, B * B
C1 = 1.0 / (2.0 * (1.0 - A2) * (1.0 - B2))
CA = 1.0 / (2.0 * A2 * (A2 - 1.0) * (A2 - B2))
CB = 1.0 / (2.0 * B2 * (B2 - 1.0) * (B2 - A2))
NP = 8


def _input_transform(d0, d1, d2, d3, d4, d5, d6, d7):
    d64, d42, d53, d31 = d6 - d4, d4 - d2, d5 - d3, d3 - d1
    v0 = (d0 - d6) + (A2 + 1.0 + B2) * d42
    v7 = (d7 - d1) - (A2 + 1.0 + B2) * d53
    e1 = (d6 + d2) - (A2 + B2) * d4
    o1 = (d5 + d1) - (A2 + B2) * d3
    ea, eb = d64 - B2 * d42, d64 - A2 * d42
    oa, ob = A * d53 - B * d31, B * d53 - A * d31
    return v0, e1 + o1, e1 - o1, ea + oa, ea - oa, eb + ob, eb - ob, v7


def _filter_transform(w0, w1, w2):
    e1, o1 = C1 * (w0 + w2), C1 * w1
    ea, oa = CA * w0 + (CA * A2) * w2, (CA * A) * w1
    eb, ob = CB * w0 + (CB * B2) * w2, (CB * B) * w1
    return e1 + o1, e1 - o1, ea + oa, ea - oa, eb + ob, eb - ob


def _bf(u):
    return pltpu.bitcast(u, BF16)


def _mm(a, b):
    return jnp.dot(a, b, preferred_element_type=F32)


def _cat(parts, axis):
    return parts[0] if len(parts) == 1 else jnp.concatenate(parts, axis=axis)


def make(scopes=False, lastsplit=(176, 96, 48, 32), pf=(0.0, 1.0), s0n=4, s1n=5, s2n=2, nf=33, merged=False, cf=(0.0, 0.95), gset=(1, 2, 3), pad=0, LB=4, ap=0,
         t3e=0.9, t2free=7, s2w=(0.4, 0.9), t2e=0.5, dgx=2, dgw=2, s1t=0.6,
         s1w=(0.2, 0.8), MA=192, tb=(0.0, 0.2), wb=(0.2, 0.9)):
    scope = jax.named_scope if scopes else (lambda n: contextlib.nullcontext())
    order = (1, 2, 3, 4, 5, 6, 0, 7)

    @jax.jit
    def f(x, w, mean, var, g, b):
        _, S, C = x.shape
        assert x.shape == (2, 2048, 1024) and w.shape == (3, C, C)
        NC = C // 128
        KH = C // 2
        PADF, GAP = 16, 8
        B1 = S + GAP
        MT = (336, 352)
        T0 = (0, MT[0])
        NT = sum(MT)
        XR = PADF + 6 * NT + 24
        OR = 6 * NT + 16
        RA = 6 * MA + 16

        def kern(x_hbm, w_hbm, m_hbm, v_hbm, g_hbm, b_hbm, o_hbm,
                 xs, osb, wl, wh, acc, bns, junk, pm, pv, pg, pb, xsem, wsem, osem, psem, *bufs):
            ug, uh = bufs[0:6], bufs[6:8]
            vs = (bufs[8:8 + NC], bufs[8 + NC:8 + 2 * NC])
            xs32, os32, wh32 = xs.bitcast(U32), osb.bitcast(U32), wh.bitcast(U32)

            def xrows(bb, c, r0, n, s):
                return pltpu.make_async_copy(x_hbm.at[bb, pl.ds(r0, n), pl.ds(c * 128, 128)],
                                             xs.at[c, pl.ds(PADF + bb * B1 + r0, n), :], xsem.at[s])

            def xcols(bb, cs, s):
                return [xrows(bb, c, 0, S, s) for c in cs]

            def wrows(k, s):
                return [pltpu.make_async_copy(w_hbm.at[:, pl.ds(k * 128, 128), :], wl.at[:, pl.ds(k * 128, 128), :],
                                              wsem.at[s])]

            def whalf(k, h, s):
                return [pltpu.make_async_copy(w_hbm.at[t, pl.ds(k * 128, 128), pl.ds(h * KH, KH)],
                                              wl.at[t, pl.ds(k * 128, 128), pl.ds(h * KH, KH)], wsem.at[s])
                        for t in range(3)]

            def whigh(js, s):
                return [pltpu.make_async_copy(w_hbm.at[t, pl.ds(KH, KH), pl.ds(j * 128, 128)], wh.at[j, t], wsem.at[s])
                        for j in js for t in range(3)]

            def orows(bb, c, r0, n):
                col = c * 128 if isinstance(c, int) else pl.multiple_of(c * 128, 128)
                return pltpu.make_async_copy(osb.at[c, pl.ds(bb * B1 + r0, n), :],
                                             o_hbm.at[bb, pl.ds(r0, n), pl.ds(col, 128)], osem.at[0])

            def send(c, t0, t1):
                for bb in range(2):
                    lo, hi = max(6 * t0, bb * B1), min(6 * t1, bb * B1 + S)
                    if hi > lo:
                        orows(bb, c, lo - bb * B1, hi - lo).start(priority=1)

            def start(cs):
                for cp in cs:
                    cp.start()

            def wait(cs):
                for cp in cs:
                    cp.wait()

            g_w1 = whalf(0, 0, 4)
            g_xa0 = [xrows(0, 0, 0, RA, 0)]
            g_w2 = whalf(0, 1, 5) + [xrows(0, 0, RA, S - RA, 5)]
            g_k1 = xcols(0, [1], 1) + wrows(1, 1)
            g_k23 = xcols(0, [2, 3], 2) + wrows(2, 2) + whalf(3, 0, 2)
            g_x1 = xcols(1, range(4), 3) + whalf(3, 1, 3)
            g_par = [pltpu.make_async_copy(src, dst, psem.at[0])
                     for src, dst in ((m_hbm, pm), (v_hbm, pv), (g_hbm, pg), (b_hbm, pb))]
            g_rest = xcols(0, range(4, NC), 4) + xcols(1, range(4, NC), 4) + whigh(range(NC), 0) + g_par

            def runtime_zero(seed):
                return jax.lax.fori_loop(0, 6, lambda i, c: c >> 1, seed)

            start(g_w1)
            zero = runtime_zero(21)
            start(g_xa0)
            zero = zero + runtime_zero(19)
            start(g_w2)
            zero = zero + runtime_zero(17)
            start(g_k1)
            for c in range(NC):
                for r0, r1 in ((0, PADF), (PADF + S, PADF + B1), (PADF + B1 + S, XR)):
                    xs[c, pl.ds(r0, r1 - r0), :] = jnp.zeros((r1 - r0, 128), BF16)

            if pad:
                @pl.when(zero != 0)
                def _():
                    for k in range(pad):
                        os32[k % NC, pl.ds(8 * (k // NC), 8), :] = jnp.full((8, 128), k, U32)

            views = {}

            def shifted(buf):
                if id(buf) not in views:
                    rows = pl.ds(pl.multiple_of(zero, 16), buf.shape[-2])
                    views[id(buf)] = buf.at[(slice(None),) * (len(buf.shape) - 2) + (rows, slice(None))]
                return views[id(buf)]

            def hold(v, gate):
                return jnp.where(jnp.full((8, 128), zero, jnp.int32) == 0, v, pltpu.bitcast(gate, v.dtype))

            def place(items, gates, f0, f1):
                for k, item in enumerate(items):
                    gi = int(len(gates) * (f0 + (f1 - f0) * k / len(items)))

                    def gate(d, gi=gi):
                        arr, r = gates[min(gi + d, len(gates) - 1)]
                        return arr[r:r + 8, 0:128]
                    item(gate)

            def free(items):
                for item in items:
                    item(None)

            def u_at(j, i, k):
                if k >= 4:
                    return uh[j[1] % 2], (i,), 4
                if k == 0:
                    return ug[j // 4], (j % 4, i - 1), 0
                if k == 1:
                    return ug[2], (j, i - 1), 1
                if j < 4:
                    return ug[3], (j, i - 1), 2
                return ug[2 + k], (j - 4, i - 1), k

            def w_item(j, r0, gate):
                if r0 >= KH:
                    raw = [wh32[j[0] * LB + j[1], t, pl.ds((r0 - KH) // 2, 8), :] for t in range(3)]
                else:
                    raw = [pltpu.bitcast(wl[t, pl.ds(r0, 16), pl.ds(j * 128, 128)], U32) for t in range(3)]
                if gate is None:
                    us = _filter_transform(*(_bf(u).astype(F32) for u in raw))
                else:
                    top = _filter_transform(*(_bf(hold(u, gate(0))).astype(F32)[0:8] for u in raw))
                    bot = _filter_transform(*(_bf(hold(u, gate(dgw))).astype(F32)[8:16] for u in raw))
                    us = [_cat(p, 0) for p in zip(top, bot)]
                for i in range(1, 7):
                    buf, idx, kb = u_at(j, i, r0 // 128)
                    shifted(buf)[idx + (pl.ds(r0 - 128 * kb, 16), slice(None))] = us[i - 1].astype(BF16)
                if r0 >= KH:
                    for i, t in ((0, 0), (7, 2)):
                        u = raw[t] if gate is None else hold(raw[t], gate(0))
                        shifted(uh[j[1] % 2])[i, pl.ds(r0 - KH, 16), :] = _bf(u)

            def w_items(js, k0, k1):
                return [functools.partial(w_item, j, r0) for j in js for r0 in range(k0 * 128, k1 * 128, 16)]

            def unpackers(gate, d):
                mask, shift = jnp.full((8, 128), 0xFFFF0000, U32), jnp.full((8, 128), 16, U32)
                if gate is not None:
                    mask, shift = hold(mask, gate(d)), hold(shift, gate(d))
                return (lambda u: pltpu.bitcast(u << shift, F32)), (lambda u: pltpu.bitcast(u & mask, F32))

            v_first = [[] for _ in range(NP)]

            def x_item(ch, c, t0, gate):
                base = PADF // 2 + 3 * (T0[ch] + t0)
                u = [xs32[c, pl.ds(base + o, 8, stride=6), :] for o in range(-1, 7)]
                lo, hi = unpackers(gate, 0)
                d = [hi(u[0]), lo(u[1]), hi(u[1]), lo(u[2]), hi(u[2]), lo(u[3]), hi(u[3]), lo(u[4])]
                lo, hi = unpackers(gate, dgx)
                d += [hi(u[4]), lo(u[5]), hi(u[5]), lo(u[6]), hi(u[6]), lo(u[7])]
                even, odd = _input_transform(*d[0:8]), _input_transform(*d[6:14])
                for i in range(NP):
                    if ch == 0 and c == 0 and t0 < MA:
                        v_first[i] += [even[i], odd[i]]
                    else:
                        shifted(vs[ch][c])[i, pl.ds(t0, 16), :] = _cat([even[i], odd[i]], 0).astype(BF16)

            def x_items(ch, cs):
                return [functools.partial(x_item, ch, c, t0) for c in cs for t0 in range(0, MT[ch], 16)]

            def epilogue(M, c, m0, m1):
                sc, sh = bns[c, 0], bns[c, 1]
                ka, kb = [A ** k * sc for k in range(6)], [B ** k * sc for k in range(6)]
                for r0 in range(0, m1 - m0, 16):
                    m = [q[r0:r0 + 16] for q in M]
                    two = lambda v: _cat([v, v], 0)
                    p1 = ((m[1] + m[2]) * two(sc) + two(sh), (m[1] - m[2]) * two(sc) + two(sh))
                    pa, pb_ = (m[3] + m[4], m[3] - m[4]), (m[5] + m[6], m[5] - m[6])
                    kk = [two(hold(ka[k], m[5][0:8]) if k % 2 else ka[k]) for k in range(6)]
                    h = [(p1[k % 2] + pa[k % 2] * kk[k]) + pb_[k % 2] * two(kb[k]) for k in range(6)]
                    h[0] = h[0] + m[0] * two(sc)
                    h[5] = h[5] + m[7] * two(sc)
                    for k, i in ((1, 0), (4, 7)):
                        h[k] = _cat([hold(h[k][e:e + 8], m[i][e:e + 8]) for e in (0, 8)], 0)
                    o = [pltpu.bitcast(q * jnp.tanh(q) + q, U32) + jnp.uint32(0x8000) for q in h]
                    for p in range(3):
                        words = (o[2 * p] >> 16) | (o[2 * p + 1] & jnp.uint32(0xFFFF0000))
                        for par in range(2):
                            row = 3 * (m0 + r0 + par) + p
                            os32[c, pl.ds(row, 8, stride=6), :] = words[8 * par:8 * par + 8]

            def u_load(i, k0, k1, j0, j1):
                if i in (0, 7):
                    return wl[0 if i == 0 else 2, k0 * 128:k1 * 128, j0 * 128:j1 * 128]

                def col(j):
                    ks = [k for k in range(k0, k1) if u_at(j, i, k)[2] == k]
                    return _cat([u_at(j, i, k)[0].bitcast(U32)[u_at(j, i, k)[1]] for k in ks], 0)
                return _bf(_cat([col(j) for j in range(j0, j1)], 1))

            def v_load(ch, i, k0, k1, m0, m1):
                return _bf(_cat([vs[ch][c].bitcast(U32)[i, m0 // 2:m1 // 2, :] for c in range(k0, k1)], 1))

            def rows8(r):
                return [(r, rr) for rr in range(0, r.shape[0], 8)]

            v0_bf16 = {}

            def dots_0(idx, part, h):
                m0, m1 = (0, MA) if part == 0 else (MA, MT[0])
                gates = []
                for i in idx:
                    if part == 0 and i not in v0_bf16:
                        v0_bf16[i] = _cat(v_first[i], 0).astype(BF16)
                    lhs = v0_bf16[i] if part == 0 else v_load(0, i, 0, 1, m0, m1)
                    r = _mm(lhs, u_load(i, 0, 1, 4 * h, 4 * h + 4))
                    for j in range(4):
                        acc[4 * h + j, i, m0:m1, :] = r[:, j * 128:(j + 1) * 128]
                    gates += rows8(r)
                return gates

            def dots_a(idx, k0, k1, j0=0, j1=NC):
                gw = 4 // (k1 - k0)
                gates = []
                for i in idx:
                    lhs = v_load(0, i, k0, k1, 0, MT[0])
                    for j in range(j0, j1, gw):
                        r = (_cat([acc[j + q, i, 0:MT[0], :] for q in range(gw)], 1)
                             + _mm(lhs, u_load(i, k0, k1, j, j + gw)))
                        for q in range(gw):
                            acc[j + q, i, 0:MT[0], :] = r[:, q * 128:(q + 1) * 128]
                        gates += rows8(r)
                return gates

            def block(j, t0, t1):
                M, gates = [None] * NP, []
                for i in order:
                    lhs = _cat([v_load(ch, i, 4, NC, max(t0, T0[ch]) - T0[ch], min(t1, T0[ch] + MT[ch]) - T0[ch])
                                for ch in range(2) if max(t0, T0[ch]) < min(t1, T0[ch] + MT[ch])], 0)
                    c = j[0] * LB + j[1]
                    rhs = uh[j[1] % 2].bitcast(U32)[i]
                    M[i] = acc[c, i, t0:t1, :] + _mm(lhs, _bf(rhs))
                    if i in gset:
                        gates += rows8(M[i])
                return M, gates

            lo_j, hi_j = range(4), range(4, NC)
            with scope('w_w1'):
                wait(g_w1)
            with scope('W1'):
                start(g_k23)
                free(w_items(lo_j, 0, 1))
            with scope('w_xa0'):
                wait(g_xa0)
            x0 = x_items(0, [0])
            with scope('S2'):
                free(x0[:MA // 16])
                dots_0(range(NP), 0, 0)
            with scope('w_w2'):
                wait(g_w2)
            with scope('s0'):
                gt = dots_0((0, 7), 0, 1)
                free(x0[MA // 16:MA // 16 + 3])
                place(x0[MA // 16 + 3:], gt, *tb)
                gt += dots_0(range(NP), 1, 0)
                place(w_items(hi_j, 0, 1), gt, *wb)
                dots_0((0, 7), 1, 1)
                for i in range(1, s0n + 1):
                    dots_0((i,), 0, 1), dots_0((i,), 1, 1)
                start(g_x1)
            with scope('w_k1'):
                wait(g_k1)
            with scope('s1'):
                gt = []
                for i in range(s0n + 1, 7):
                    gt += dots_0((i,), 0, 1) + dots_0((i,), 1, 1)
                place(x_items(0, [1]), gt, 0.0, s1t)
                gt += dots_a((0, 7), 1, 2)
                place(w_items(range(NC), 1, 2), gt, *s1w)
                dots_a(range(1, s1n + 1), 1, 2)
            with scope('w_k23'):
                wait(g_k23)
            with scope('s2'):
                gt = dots_a(range(s1n + 1, 7), 1, 2)
                x2 = x_items(0, [2])
                free(x2[:t2free])
                place(x2[t2free:], gt, 0.0, t2e)
                gt = dots_a((0, 7), 2, 3)
                place(x_items(0, [3]), gt, 0.0, t3e)
                gt += dots_a((0, 7), 3, 4, 0, 4)
                place(w_items(hi_j, 2, 3), gt, *s2w)
                gt = dots_a(range(1, 7), 2, 3, 4, NC)
                place(w_items(lo_j, 2, 4), gt, 0.0, 0.9)
                dots_a(range(1, s2n + 1), 2, 4, 0, 4)
                start(g_rest)
            with scope('w_x1'):
                wait(g_x1)
            with scope('s3'):
                gt = dots_a(range(s2n + 1, 7), 2, 4, 0, 4) + dots_a((0, 7), 3, 4, 4, NC)
                place(w_items(hi_j, 3, 4), gt, 0.0, 0.8)
                gt += dots_a(range(1, 7), 3, 4, 4, NC)
                place(x_items(1, range(4)), gt, 0.0, 0.92)

                gt = []
                for n in range(NC * NP):
                    if n == nf:
                        with scope('w_rest'):
                            wait(g_rest)
                        gt = []
                    j, i = divmod(n, NP)
                    r = _mm(v_load(1, i, 0, 4, 0, MT[1]), u_load(i, 0, 4, j, j + 1))
                    acc[j, i, MT[0]:NT, :] = r
                    gt += rows8(r)
                mean_, var_, g_, b_ = (p[...].astype(F32).reshape(1, C) for p in (pm, pv, pg, pb))
                scale = g_ * jax.lax.rsqrt(var_ + 1e-5)
                for q, p in enumerate((0.5 * scale, 0.5 * (b_ - mean_ * scale))):
                    for j in range(NC):
                        bns[j, q] = jnp.broadcast_to(p[:, j * 128:(j + 1) * 128], (8, 128))
                place(x_items(0, range(4, NC)) + x_items(1, range(4, NC)), gt, *cf)
                place(w_items([(0, 0)], 4, NC), gt, *cf)

            with scope('B'):
                def blocks(it, carry):
                    views.clear()
                    for jj in range(LB):
                        cuts = [0, MT[0]]
                        if jj == LB - 1:
                            cuts += [NT - sum(lastsplit[k:]) for k in range(1, len(lastsplit))]
                        gt = []
                        for t0, t1 in zip(cuts, cuts[1:] + [NT]):
                            M, gates = block((it, jj), t0, t1)
                            gt += gates
                            epilogue(M, it * LB + jj, t0, t1)
                            send(it * LB + jj, t0, t1)
                        nxt = (it, jj + 1) if jj + 1 < LB else ((it + 1) % (NC // LB), 0)
                        place(w_items([nxt], 4, NC), gt, *pf)
                    return carry
                jax.lax.fori_loop(0, NC // LB, blocks, 0)
            with scope('w_out'):
                wait([orows(bb, c, 0, S) for bb in range(2) for c in range(NC)])

        vmem = pltpu.VMEM
        return pl.pallas_call(
            kern,
            in_specs=[pl.BlockSpec(memory_space=pl.ANY)] * 6,
            out_specs=pl.BlockSpec(memory_space=pl.ANY),
            out_shape=jax.ShapeDtypeStruct(x.shape, x.dtype),
            scratch_shapes=[
                vmem((NC, XR, 128), BF16), vmem((NC, OR, 128), BF16),
                vmem((3, KH, C), BF16), vmem((NC, 3, KH, 128), BF16),
                vmem((NC, NP, NT + ap, 128), F32), vmem((NC, 2, 8, 128), F32), vmem((8 * max(pad, 1), 128), F32),
                vmem((C,), BF16), vmem((C,), BF16), vmem((C,), BF16), vmem((C,), BF16),
                pltpu.SemaphoreType.DMA((6,)), pltpu.SemaphoreType.DMA((6,)),
                pltpu.SemaphoreType.DMA((1,)), pltpu.SemaphoreType.DMA((1,)),
                vmem((4, 6, 128, 128), BF16), vmem((4, 6, 128, 128), BF16), vmem((NC, 6, 128, 128), BF16),
                vmem((4, 6, 256, 128), BF16), vmem((4, 6, 128, 128), BF16), vmem((4, 6, 128, 128), BF16),
            ] + [vmem((NP, KH, 128), BF16)] * 2 + [vmem((NP, MT[0], 128), BF16)] * NC + [vmem((NP, MT[1], 128), BF16)] * NC,
            compiler_params=pltpu.CompilerParams(vmem_limit_bytes=110 * 2 ** 20, disable_bounds_checks=True,
                                                 disable_semaphore_checks=True),
        )(x, w, mean, var, g, b)
    return f


pallas_standalone__batchnorm__prompt_kernel = make()
```

```python
import contextlib
import functools

import jax
import jax.numpy as jnp
import jax.experimental.pallas as pl
import jax.experimental.pallas.tpu as pltpu

F32, U32, BF16 = jnp.float32, jnp.uint32, jnp.bfloat16

A = 0.52
B = 1.0 / A
A2, B2 = A * A, B * B
C1 = 1.0 / (2.0 * (1.0 - A2) * (1.0 - B2))
CA = 1.0 / (2.0 * A2 * (A2 - 1.0) * (A2 - B2))
CB = 1.0 / (2.0 * B2 * (B2 - 1.0) * (B2 - A2))
NP = 8


def _input_transform(d0, d1, d2, d3, d4, d5, d6, d7):
    d64, d42, d53, d31 = d6 - d4, d4 - d2, d5 - d3, d3 - d1
    v0 = (d0 - d6) + (A2 + 1.0 + B2) * d42
    v7 = (d7 - d1) - (A2 + 1.0 + B2) * d53
    e1 = (d6 + d2) - (A2 + B2) * d4
    o1 = (d5 + d1) - (A2 + B2) * d3
    ea, eb = d64 - B2 * d42, d64 - A2 * d42
    oa, ob = A * d53 - B * d31, B * d53 - A * d31
    return v0, e1 + o1, e1 - o1, ea + oa, ea - oa, eb + ob, eb - ob, v7


def _filter_transform(w0, w1, w2):
    e1, o1 = C1 * (w0 + w2), C1 * w1
    ea, oa = CA * w0 + (CA * A2) * w2, (CA * A) * w1
    eb, ob = CB * w0 + (CB * B2) * w2, (CB * B) * w1
    return e1 + o1, e1 - o1, ea + oa, ea - oa, eb + ob, eb - ob


def _bf(u):
    return pltpu.bitcast(u, BF16)


def _mm(a, b):
    return jnp.dot(a, b, preferred_element_type=F32)


def _cat(parts, axis):
    return parts[0] if len(parts) == 1 else jnp.concatenate(parts, axis=axis)


def make(scopes=False, lastsplit=(176, 96, 48, 32), MQ=112, MA=208, dgx=2, dgw=2, tb=(0.0, 0.2), wb=(0.2, 0.9),
         qw=(0.2, 0.8), s0n=6, s1n=4, s3n=2, e1=0.8, e2=0.85, e3=0.85, LB=4, f1=0.2):
    scope = jax.named_scope if scopes else (lambda n: contextlib.nullcontext())
    order = (1, 2, 3, 4, 5, 6, 0, 7)

    @jax.jit
    def f(x, w, mean, var, g, b):
        _, S, C = x.shape
        assert x.shape == (2, 2048, 1024) and w.shape == (3, C, C)
        NC = C // 128
        KH = C // 2
        PADF, GAP = 16, 8
        B1 = S + GAP
        MT = (336, 352)
        T0 = (0, MT[0])
        NT = sum(MT)
        XR = PADF + 6 * NT + 24
        OR = 6 * NT + 16
        RQ, RA = 6 * MQ + 16, 6 * MA + 16

        def kern(x_hbm, w_hbm, m_hbm, v_hbm, g_hbm, b_hbm, o_hbm,
                 xs, osb, wl, wh, acc, bns, pm, pv, pg, pb, xsem, wsem, osem, psem, *bufs):
            ul, uh = bufs[0:6], bufs[6:8]
            vs = (bufs[8:8 + NC], bufs[8 + NC:8 + 2 * NC])
            xs32, os32, wh32 = xs.bitcast(U32), osb.bitcast(U32), wh.bitcast(U32)

            def xrows(bb, c, r0, n, s):
                return pltpu.make_async_copy(x_hbm.at[bb, pl.ds(r0, n), pl.ds(c * 128, 128)],
                                             xs.at[c, pl.ds(PADF + bb * B1 + r0, n), :], xsem.at[s])

            def xcols(bb, cs, s):
                return [xrows(bb, c, 0, S, s) for c in cs]

            def wrows(k, s):
                return [pltpu.make_async_copy(w_hbm.at[:, pl.ds(k * 128, 128), :], wl.at[:, pl.ds(k * 128, 128), :],
                                              wsem.at[s])]

            def wpart(j0, j1, s):
                cols = pl.ds(j0 * 128, (j1 - j0) * 128)
                return [pltpu.make_async_copy(w_hbm.at[t, pl.ds(0, 128), cols], wl.at[t, pl.ds(0, 128), cols],
                                              wsem.at[s]) for t in range(3)]

            def whigh(s):
                return [pltpu.make_async_copy(w_hbm.at[t, pl.ds(KH, KH), pl.ds(j * 128, 128)], wh.at[j, t], wsem.at[s])
                        for j in range(NC) for t in range(3)]

            def orows(bb, c, r0, n):
                col = c * 128 if isinstance(c, int) else pl.multiple_of(c * 128, 128)
                return pltpu.make_async_copy(osb.at[c, pl.ds(bb * B1 + r0, n), :],
                                             o_hbm.at[bb, pl.ds(r0, n), pl.ds(col, 128)], osem.at[0])

            def send(c, t0, t1):
                for bb in range(2):
                    lo, hi = max(6 * t0, bb * B1), min(6 * t1, bb * B1 + S)
                    if hi > lo:
                        orows(bb, c, lo - bb * B1, hi - lo).start()

            def start(cs):
                for cp in cs:
                    cp.start()

            def wait(cs):
                for cp in cs:
                    cp.wait()

            g_w1 = wpart(0, 2, 0)
            g_x1 = [xrows(0, 0, 0, RQ, 0)]
            g_q = wpart(2, 4, 1) + [xrows(0, 0, RQ, RA - RQ, 1)]
            g_w2 = wpart(4, NC, 2) + [xrows(0, 0, RA, S - RA, 2)]
            g_b2 = xcols(1, [0], 3) + xcols(0, [1], 3) + wrows(1, 3)
            g_b3 = xcols(1, [1, 2, 3], 4) + xcols(0, [2, 3], 4) + wrows(2, 4) + wrows(3, 4)
            g_rest = xcols(0, range(4, NC), 5) + xcols(1, range(4, NC), 5) + whigh(5) + [
                pltpu.make_async_copy(src, dst, psem.at[0])
                for src, dst in ((m_hbm, pm), (v_hbm, pv), (g_hbm, pg), (b_hbm, pb))]

            def runtime_zero(seed):
                return jax.lax.fori_loop(0, 5, lambda i, c: c >> 1, seed)

            zero = 0
            for n, group in enumerate((g_w1, g_x1, g_q, g_w2)):
                start(group)
                zero = zero + runtime_zero(17 + 2 * n)
            start(g_b2)
            for c in range(NC):
                for r0, r1 in ((0, PADF), (PADF + S, PADF + B1), (PADF + B1 + S, XR)):
                    xs[c, pl.ds(r0, r1 - r0), :] = jnp.zeros((r1 - r0, 128), BF16)

            views = {}

            def shifted(buf):
                if id(buf) not in views:
                    rows = pl.ds(pl.multiple_of(zero, 16), buf.shape[-2])
                    views[id(buf)] = buf.at[(slice(None),) * (len(buf.shape) - 2) + (rows, slice(None))]
                return views[id(buf)]

            def hold(v, gate):
                return jnp.where(jnp.full((8, 128), zero, jnp.int32) == 0, v, pltpu.bitcast(gate, v.dtype))

            def place(items, gates, f0, f1):
                for k, item in enumerate(items):
                    gi = int(len(gates) * (f0 + (f1 - f0) * k / len(items)))

                    def gate(d, gi=gi):
                        arr, r = gates[min(gi + d, len(gates) - 1)]
                        return arr[r:r + 8, 0:128]
                    item(gate)

            def free(items):
                for item in items:
                    item(None)

            def u_low(j, k):
                if k > 0:
                    return ul[2 + k], j
                return (ul[0], j) if j < 2 else (ul[1], j - 2) if j < 4 else (ul[2], j - 4)

            def filter16(raw, gate):
                if gate is None:
                    return _filter_transform(*(_bf(u).astype(F32) for u in raw))
                top = _filter_transform(*(_bf(hold(u, gate(0))).astype(F32)[0:8] for u in raw))
                bot = _filter_transform(*(_bf(hold(u, gate(dgw))).astype(F32)[8:16] for u in raw))
                return [_cat(p, 0) for p in zip(top, bot)]

            def wl_item(j, r0, gate):
                raw = [pltpu.bitcast(wl[t, pl.ds(r0, 16), pl.ds(j * 128, 128)], U32) for t in range(3)]
                buf, slot = u_low(j, r0 // 128)
                for i, u in enumerate(filter16(raw, gate)):
                    shifted(buf)[slot, i, pl.ds(r0 % 128, 16), :] = u.astype(BF16)

            def wl_items(js, k0, k1):
                return [functools.partial(wl_item, j, r0) for j in js for r0 in range(k0 * 128, k1 * 128, 16)]

            def wh_item(j, buf, r0, gate):
                raw = [wh32[j, t, pl.ds(r0 // 2, 8), :] for t in range(3)]
                us = [u.astype(BF16) for u in filter16(raw, gate)]
                for i, u in enumerate([_bf(hold(raw[0], gate(0)))] + us + [_bf(hold(raw[2], gate(0)))]):
                    shifted(buf)[i, pl.ds(r0, 16), :] = u

            def wh_items(j, buf):
                return [functools.partial(wh_item, j, buf, r0) for r0 in range(0, KH, 16)]

            def unpackers(gate, d):
                mask, shift = jnp.full((8, 128), 0xFFFF0000, U32), jnp.full((8, 128), 16, U32)
                if gate is not None:
                    mask, shift = hold(mask, gate(d)), hold(shift, gate(d))
                return (lambda u: pltpu.bitcast(u << shift, F32)), (lambda u: pltpu.bitcast(u & mask, F32))

            v_first = [[[] for _ in range(NP)] for _ in range(2)]

            def x_item(ch, c, t0, gate):
                base = PADF // 2 + 3 * (T0[ch] + t0)
                u = [xs32[c, pl.ds(base + o, 8, stride=6), :] for o in range(-1, 7)]
                lo, hi = unpackers(gate, 0)
                d = [hi(u[0]), lo(u[1]), hi(u[1]), lo(u[2]), hi(u[2]), lo(u[3]), hi(u[3]), lo(u[4])]
                lo, hi = unpackers(gate, dgx)
                d += [hi(u[4]), lo(u[5]), hi(u[5]), lo(u[6]), hi(u[6]), lo(u[7])]
                even, odd = _input_transform(*d[0:8]), _input_transform(*d[6:14])
                for i in range(NP):
                    if c == 0 and ((ch == 0 and t0 < MA) or (ch == 1 and s0n == 6)):
                        v_first[ch][i] += [even[i], odd[i]]
                    else:
                        shifted(vs[ch][c])[i, pl.ds(t0, 16), :] = _cat([even[i], odd[i]], 0).astype(BF16)

            def x_items(ch, cs):
                return [functools.partial(x_item, ch, c, t0) for c in cs for t0 in range(0, MT[ch], 16)]

            def epilogue(M, c, m0, m1):
                sc, sh = bns[c, 0], bns[c, 1]
                ka, kb = [A ** k * sc for k in range(6)], [B ** k * sc for k in range(6)]

                def two(v):
                    return _cat([v, v], 0)
                for r0 in range(0, m1 - m0, 16):
                    m = [q[r0:r0 + 16] for q in M]
                    p1 = ((m[1] + m[2]) * two(sc) + two(sh), (m[1] - m[2]) * two(sc) + two(sh))
                    pa, pb_ = (m[3] + m[4], m[3] - m[4]), (m[5] + m[6], m[5] - m[6])
                    kk = [two(hold(ka[k], m[5][0:8]) if k % 2 else ka[k]) for k in range(6)]
                    h = [(p1[k % 2] + pa[k % 2] * kk[k]) + pb_[k % 2] * two(kb[k]) for k in range(6)]
                    h[0] = h[0] + m[0] * two(sc)
                    h[5] = h[5] + m[7] * two(sc)
                    for k, i in ((1, 0), (4, 7)):
                        h[k] = _cat([hold(h[k][e:e + 8], m[i][e:e + 8]) for e in (0, 8)], 0)
                    o = [pltpu.bitcast(q * jnp.tanh(q) + q, U32) + jnp.uint32(0x8000) for q in h]
                    for p in range(3):
                        words = (o[2 * p] >> 16) | (o[2 * p + 1] & jnp.uint32(0xFFFF0000))
                        for par in range(2):
                            os32[c, pl.ds(3 * (m0 + r0 + par) + p, 8, stride=6), :] = words[8 * par:8 * par + 8]

            def u_load(i, k0, k1, j0, j1):
                if i in (0, 7):
                    return wl[0 if i == 0 else 2, k0 * 128:k1 * 128, j0 * 128:j1 * 128]
                return _bf(_cat([_cat([u_low(j, k)[0].bitcast(U32)[u_low(j, k)[1], i - 1] for k in range(k0, k1)], 0)
                                 for j in range(j0, j1)], 1))

            def v_load(ch, i, k0, k1, m0, m1):
                return _bf(_cat([vs[ch][c].bitcast(U32)[i, m0 // 2:m1 // 2, :] for c in range(k0, k1)], 1))

            def rows8(r):
                return [(r, rr) for rr in range(0, r.shape[0], 8)]

            v0_bf16 = {}

            def dots_0(idx, m0, m1, j0, j1):
                gates = []
                for i in idx:
                    if m1 <= MA:
                        parts = [(p0, p1) for p0, p1 in ((0, MQ), (MQ, MA)) if m0 <= p0 < m1]
                        for p0, p1 in parts:
                            if (i, p0) not in v0_bf16:
                                v0_bf16[i, p0] = _cat(v_first[0][i][p0 // 8:p1 // 8], 0).astype(BF16)
                        lhs = _cat([v0_bf16[i, p0] for p0, _ in parts], 0)
                    else:
                        lhs = v_load(0, i, 0, 1, m0, m1)
                    r = _mm(lhs, u_load(i, 0, 1, j0, j1))
                    for j in range(j0, j1):
                        acc[j, i, m0:m1, :] = r[:, (j - j0) * 128:(j - j0 + 1) * 128]
                    gates += rows8(r)
                return gates

            def dots(ch, idx, k0, k1):
                gw = 4 // (k1 - k0)
                rows = slice(T0[ch], T0[ch] + MT[ch])
                gates = []
                for i in idx:
                    if k0 == 0 and s0n == 6:
                        lhs = _cat(v_first[ch][i], 0).astype(BF16)
                    else:
                        lhs = v_load(ch, i, k0, k1, 0, MT[ch])
                    for j in range(0, NC, gw):
                        r = _mm(lhs, u_load(i, k0, k1, j, j + gw))
                        if k0 > 0:
                            r = _cat([acc[j + q, i, rows, :] for q in range(gw)], 1) + r
                        for q in range(gw):
                            acc[j + q, i, rows, :] = r[:, q * 128:(q + 1) * 128]
                        gates += rows8(r)
                return gates

            with scope('w_w1'):
                wait(g_w1)
            with scope('W1'):
                start(g_b3)
                free(wl_items(range(2), 0, 1))
            with scope('w_x1'):
                wait(g_x1)
            x0 = x_items(0, [0])
            with scope('S1'):
                free(x0[:MQ // 16])
                dots_0(range(NP), 0, MQ, 0, 2)
            with scope('w_q'):
                wait(g_q)
            with scope('S2'):
                free(x0[MQ // 16:MA // 16])
                gt = dots_0((0, 7), 0, MQ, 2, 4) + dots_0(range(NP), MQ, MA, 0, 2)
                place(wl_items(range(2, 4), 0, 1), gt, *qw)
                dots_0((0, 7), MQ, MA, 2, 4)
                dots_0(range(1, 7), 0, MA, 2, 4)
            with scope('w_w2'):
                wait(g_w2)
            with scope('s0'):
                gt = dots_0((0, 7), 0, MA, 4, NC)
                free(x0[MA // 16:MA // 16 + 3])
                place(x0[MA // 16 + 3:], gt, *tb)
                gt += dots_0(range(NP), MA, MT[0], 0, 4)
                place(wl_items(range(4, NC), 0, 1), gt, *wb)
                dots_0((0, 7), MA, MT[0], 4, NC)
                for i in range(1, s0n + 1):
                    dots_0((i,), 0, MA, 4, NC), dots_0((i,), MA, MT[0], 4, NC)
            with scope('w_b2'):
                wait(g_b2)
            with scope('s1'):
                gt = []
                for i in range(s0n + 1, 7):
                    gt += dots_0((i,), 0, MA, 4, NC) + dots_0((i,), MA, MT[0], 4, NC)
                if gt:
                    place(x_items(1, [0]), gt, 0.0, e1)
                else:
                    free(x_items(1, [0]))
                gt = dots(1, range(NP), 0, 1)
                place(x_items(0, [1]) + wl_items(range(NC), 1, 2), gt, f1, 0.95)
                dots(0, (0, 7, 1, 2, 3, 4, 5, 6)[:s1n + 2], 1, 2)
                start(g_rest)
            with scope('w_b3'):
                wait(g_b3)
            with scope('s2'):
                gt = dots(0, range(s1n + 1, 7), 1, 2)
                place(x_items(1, [1]), gt, 0.0, e2)
                gt = dots(1, range(NP), 1, 2)
                place(x_items(0, [2, 3]) + wl_items(range(NC), 2, 4), gt, 0.0, 0.97)
                gt = dots(0, range(NP - s3n), 2, 4)
                place(x_items(1, [2, 3]), gt, 0.0, e3)
            with scope('w_rest'):
                wait(g_rest)
            with scope('s3'):
                gt = dots(0, range(NP - s3n, NP), 2, 4) + dots(1, range(NP), 2, 4)
                mean_, var_, g_, b_ = (p[...].astype(F32).reshape(1, C) for p in (pm, pv, pg, pb))
                scale = g_ * jax.lax.rsqrt(var_ + 1e-5)
                for q, p in enumerate((0.5 * scale, 0.5 * (b_ - mean_ * scale))):
                    for j in range(NC):
                        bns[j, q] = jnp.broadcast_to(p[:, j * 128:(j + 1) * 128], (8, 128))
                place(x_items(0, range(4, NC)) + x_items(1, range(4, NC)) + wh_items(0, uh[0]), gt, 0.02, 0.98)

            def blocks(it, carry):
                views.clear()
                for jj in range(LB):
                    c = it * LB + jj
                    cuts = [0, MT[0]]
                    if jj == LB - 1:
                        cuts += [NT - sum(lastsplit[k:]) for k in range(1, len(lastsplit))]
                    gates = []
                    for t0, t1 in zip(cuts, cuts[1:] + [NT]):
                        ch = int(t0 >= T0[1])
                        M = [None] * NP
                        for i in order:
                            M[i] = acc[c, i, t0:t1, :] + _mm(v_load(ch, i, 4, NC, t0 - T0[ch], t1 - T0[ch]),
                                                             _bf(uh[jj % 2].bitcast(U32)[i]))
                            if i in (1, 2, 3):
                                gates += rows8(M[i])
                        epilogue(M, c, t0, t1)
                        send(c, t0, t1)
                    place(wh_items((c + 1) % NC, uh[(jj + 1) % 2]), gates, 0.0, 1.0)
                return carry
            with scope('B'):
                jax.lax.fori_loop(0, NC // LB, blocks, 0)
            with scope('w_out'):
                wait([orows(bb, c, 0, S) for bb in range(2) for c in range(NC)])

        vmem = pltpu.VMEM
        return pl.pallas_call(
            kern,
            in_specs=[pl.BlockSpec(memory_space=pl.ANY)] * 6,
            out_specs=pl.BlockSpec(memory_space=pl.ANY),
            out_shape=jax.ShapeDtypeStruct(x.shape, x.dtype),
            scratch_shapes=[
                vmem((NC, XR, 128), BF16), vmem((NC, OR, 128), BF16),
                vmem((3, KH, C), BF16), vmem((NC, 3, KH, 128), BF16),
                vmem((NC, NP, NT, 128), F32), vmem((NC, 2, 8, 128), F32),
                vmem((C,), BF16), vmem((C,), BF16), vmem((C,), BF16), vmem((C,), BF16),
                pltpu.SemaphoreType.DMA((6,)), pltpu.SemaphoreType.DMA((6,)),
                pltpu.SemaphoreType.DMA((1,)), pltpu.SemaphoreType.DMA((1,)),
                vmem((2, 6, 128, 128), BF16), vmem((2, 6, 128, 128), BF16), vmem((4, 6, 128, 128), BF16),
            ] + [vmem((NC, 6, 128, 128), BF16)] * 3 + [vmem((NP, KH, 128), BF16)] * 2
              + [vmem((NP, MT[0], 128), BF16)] * NC + [vmem((NP, MT[1], 128), BF16)] * NC,
            compiler_params=pltpu.CompilerParams(vmem_limit_bytes=110 * 2 ** 20, disable_bounds_checks=True,
                                                 disable_semaphore_checks=True),
        )(x, w, mean, var, g, b)
    return f


pallas_standalone__batchnorm__prompt_kernel = make()
```

```python
import contextlib
import functools

import jax
import jax.numpy as jnp
import jax.experimental.pallas as pl
import jax.experimental.pallas.tpu as pltpu

F32, U32, BF16 = jnp.float32, jnp.uint32, jnp.bfloat16

A = 0.52
B = 1.0 / A
A2, B2 = A * A, B * B
C1 = 1.0 / (2.0 * (1.0 - A2) * (1.0 - B2))
CA = 1.0 / (2.0 * A2 * (A2 - 1.0) * (A2 - B2))
CB = 1.0 / (2.0 * B2 * (B2 - 1.0) * (B2 - A2))
NP = 8


def _input_transform(d0, d1, d2, d3, d4, d5, d6, d7):
    d64, d42, d53, d31 = d6 - d4, d4 - d2, d5 - d3, d3 - d1
    v0 = (d0 - d6) + (A2 + 1.0 + B2) * d42
    v7 = (d7 - d1) - (A2 + 1.0 + B2) * d53
    e1 = (d6 + d2) - (A2 + B2) * d4
    o1 = (d5 + d1) - (A2 + B2) * d3
    ea, eb = d64 - B2 * d42, d64 - A2 * d42
    oa, ob = A * d53 - B * d31, B * d53 - A * d31
    return v0, e1 + o1, e1 - o1, ea + oa, ea - oa, eb + ob, eb - ob, v7


def _filter_transform(w0, w1, w2):
    e1, o1 = C1 * (w0 + w2), C1 * w1
    ea, oa = CA * w0 + (CA * A2) * w2, (CA * A) * w1
    eb, ob = CB * w0 + (CB * B2) * w2, (CB * B) * w1
    return e1 + o1, e1 - o1, ea + oa, ea - oa, eb + ob, eb - ob


def _bf(u):
    return pltpu.bitcast(u, BF16)


def _mm(a, b):
    return jnp.dot(a, b, preferred_element_type=F32)


def _cat(parts, axis):
    return parts[0] if len(parts) == 1 else jnp.concatenate(parts, axis=axis)


def make(scopes=False):
    scope = jax.named_scope if scopes else (lambda n: contextlib.nullcontext())

    @jax.jit
    def f(x, w, mean, var, g, b):
        _, S, C = x.shape
        assert x.shape == (2, 2048, 1024) and w.shape == (3, C, C)
        NC = C // 128
        KH = C // 2
        PADF, GAP = 16, 8
        B1 = S + GAP
        MT = (336, 352)
        T0 = (0, MT[0])
        NT = sum(MT)
        XR = PADF + 6 * NT + 24
        OR = 6 * NT + 16
        MQ, MA = 112, 208
        RQ, RA = 6 * MQ + 16, 6 * MA + 16
        LB = 4

        def kern(x_hbm, w_hbm, m_hbm, v_hbm, g_hbm, b_hbm, o_hbm,
                 xs, osb, wl, wh, acc, bns, pm, pv, pg, pb, xsem, wsem, osem, psem, *bufs):
            ul, uh = bufs[0:6], bufs[6:8]
            vs = (bufs[8:8 + NC], bufs[8 + NC:8 + 2 * NC])
            xs32, os32, wh32 = xs.bitcast(U32), osb.bitcast(U32), wh.bitcast(U32)

            def xrows(bb, c, r0, n, s):
                return pltpu.make_async_copy(x_hbm.at[bb, pl.ds(r0, n), pl.ds(c * 128, 128)],
                                             xs.at[c, pl.ds(PADF + bb * B1 + r0, n), :], xsem.at[s])

            def xcols(bb, cs, s):
                return [xrows(bb, c, 0, S, s) for c in cs]

            def wrows(k, s):
                return [pltpu.make_async_copy(w_hbm.at[:, pl.ds(k * 128, 128), :], wl.at[:, pl.ds(k * 128, 128), :],
                                              wsem.at[s])]

            def wpart(j0, j1, s):
                cols = pl.ds(j0 * 128, (j1 - j0) * 128)
                return [pltpu.make_async_copy(w_hbm.at[t, pl.ds(0, 128), cols], wl.at[t, pl.ds(0, 128), cols],
                                              wsem.at[s]) for t in range(3)]

            def whigh(s):
                return [pltpu.make_async_copy(w_hbm.at[t, pl.ds(KH, KH), pl.ds(j * 128, 128)], wh.at[j, t], wsem.at[s])
                        for j in range(NC) for t in range(3)]

            def orows(bb, c, r0, n):
                col = c * 128 if isinstance(c, int) else pl.multiple_of(c * 128, 128)
                return pltpu.make_async_copy(osb.at[c, pl.ds(bb * B1 + r0, n), :],
                                             o_hbm.at[bb, pl.ds(r0, n), pl.ds(col, 128)], osem.at[0])

            def send(c, t0, t1):
                for bb in range(2):
                    lo, hi = max(6 * t0, bb * B1), min(6 * t1, bb * B1 + S)
                    if hi > lo:
                        orows(bb, c, lo - bb * B1, hi - lo).start()

            def start(cs):
                for cp in cs:
                    cp.start()

            def wait(cs):
                for cp in cs:
                    cp.wait()

            g_w1 = wpart(0, 2, 0)
            g_x1 = [xrows(0, 0, 0, RQ, 0)]
            g_q = wpart(2, 4, 1) + [xrows(0, 0, RQ, RA - RQ, 1)]
            g_w2 = wpart(4, NC, 2) + [xrows(0, 0, RA, S - RA, 2)]
            g_b2 = xcols(1, [0], 3) + xcols(0, [1], 3) + wrows(1, 3)
            g_b3 = xcols(1, [1, 2, 3], 4) + xcols(0, [2, 3], 4) + wrows(2, 4) + wrows(3, 4)
            g_rest = xcols(0, range(4, NC), 5) + xcols(1, range(4, NC), 5) + whigh(5) + [
                pltpu.make_async_copy(src, dst, psem.at[0])
                for src, dst in ((m_hbm, pm), (v_hbm, pv), (g_hbm, pg), (b_hbm, pb))]

            def runtime_zero(seed):
                return jax.lax.fori_loop(0, 5, lambda i, c: c >> 1, seed)

            zero = 0
            for n, group in enumerate((g_w1, g_x1, g_q, g_w2)):
                start(group)
                zero = zero + runtime_zero(17 + 2 * n)
            start(g_b2)
            for c in range(NC):
                for r0, r1 in ((0, PADF), (PADF + S, PADF + B1), (PADF + B1 + S, XR)):
                    xs[c, pl.ds(r0, r1 - r0), :] = jnp.zeros((r1 - r0, 128), BF16)

            views = {}

            def shifted(buf):
                if id(buf) not in views:
                    rows = pl.ds(pl.multiple_of(zero, 16), buf.shape[-2])
                    views[id(buf)] = buf.at[(slice(None),) * (len(buf.shape) - 2) + (rows, slice(None))]
                return views[id(buf)]

            def hold(v, gate):
                return jnp.where(jnp.full((8, 128), zero, jnp.int32) == 0, v, pltpu.bitcast(gate, v.dtype))

            def place(items, gates, f0, f1):
                for k, item in enumerate(items):
                    gi = int(len(gates) * (f0 + (f1 - f0) * k / len(items)))

                    def gate(d, gi=gi):
                        arr, r = gates[min(gi + d, len(gates) - 1)]
                        return arr[r:r + 8, 0:128]
                    item(gate)

            def free(items):
                for item in items:
                    item(None)

            def u_low(j, k):
                if k > 0:
                    return ul[2 + k], j
                return (ul[0], j) if j < 2 else (ul[1], j - 2) if j < 4 else (ul[2], j - 4)

            def filter16(raw, gate):
                if gate is None:
                    return _filter_transform(*(_bf(u).astype(F32) for u in raw))
                top = _filter_transform(*(_bf(hold(u, gate(0))).astype(F32)[0:8] for u in raw))
                bot = _filter_transform(*(_bf(hold(u, gate(2))).astype(F32)[8:16] for u in raw))
                return [_cat(p, 0) for p in zip(top, bot)]

            def wl_item(j, r0, gate):
                raw = [pltpu.bitcast(wl[t, pl.ds(r0, 16), pl.ds(j * 128, 128)], U32) for t in range(3)]
                buf, slot = u_low(j, r0 // 128)
                for i, u in enumerate(filter16(raw, gate)):
                    shifted(buf)[slot, i, pl.ds(r0 % 128, 16), :] = u.astype(BF16)

            def wl_items(js, k0, k1):
                return [functools.partial(wl_item, j, r0) for j in js for r0 in range(k0 * 128, k1 * 128, 16)]

            def wh_item(j, buf, r0, gate):
                raw = [wh32[j, t, pl.ds(r0 // 2, 8), :] for t in range(3)]
                us = [u.astype(BF16) for u in filter16(raw, gate)]
                for i, u in enumerate([_bf(hold(raw[0], gate(0)))] + us + [_bf(hold(raw[2], gate(0)))]):
                    shifted(buf)[i, pl.ds(r0, 16), :] = u

            def wh_items(j, buf):
                return [functools.partial(wh_item, j, buf, r0) for r0 in range(0, KH, 16)]

            def unpackers(gate, d):
                mask, shift = jnp.full((8, 128), 0xFFFF0000, U32), jnp.full((8, 128), 16, U32)
                if gate is not None:
                    mask, shift = hold(mask, gate(d)), hold(shift, gate(d))
                return (lambda u: pltpu.bitcast(u << shift, F32)), (lambda u: pltpu.bitcast(u & mask, F32))

            v_first = [[[] for _ in range(NP)] for _ in range(2)]

            def x_item(ch, c, t0, gate):
                base = PADF // 2 + 3 * (T0[ch] + t0)
                u = [xs32[c, pl.ds(base + o, 8, stride=6), :] for o in range(-1, 7)]
                lo, hi = unpackers(gate, 0)
                d = [hi(u[0]), lo(u[1]), hi(u[1]), lo(u[2]), hi(u[2]), lo(u[3]), hi(u[3]), lo(u[4])]
                lo, hi = unpackers(gate, 2)
                d += [hi(u[4]), lo(u[5]), hi(u[5]), lo(u[6]), hi(u[6]), lo(u[7])]
                even, odd = _input_transform(*d[0:8]), _input_transform(*d[6:14])
                for i in range(NP):
                    if c == 0 and (ch == 1 or t0 < MA):
                        v_first[ch][i] += [even[i], odd[i]]
                    else:
                        shifted(vs[ch][c])[i, pl.ds(t0, 16), :] = _cat([even[i], odd[i]], 0).astype(BF16)

            def x_items(ch, cs):
                return [functools.partial(x_item, ch, c, t0) for c in cs for t0 in range(0, MT[ch], 16)]

            def epilogue(M, c, m0, m1):
                sc, sh = bns[c, 0], bns[c, 1]
                ka, kb = [A ** k * sc for k in range(6)], [B ** k * sc for k in range(6)]

                def two(v):
                    return _cat([v, v], 0)
                for r0 in range(0, m1 - m0, 16):
                    m = [q[r0:r0 + 16] for q in M]
                    p1 = ((m[1] + m[2]) * two(sc) + two(sh), (m[1] - m[2]) * two(sc) + two(sh))
                    pa, pb_ = (m[3] + m[4], m[3] - m[4]), (m[5] + m[6], m[5] - m[6])
                    kk = [two(hold(ka[k], m[5][0:8]) if k % 2 else ka[k]) for k in range(6)]
                    h = [(p1[k % 2] + pa[k % 2] * kk[k]) + pb_[k % 2] * two(kb[k]) for k in range(6)]
                    h[0] = h[0] + m[0] * two(sc)
                    h[5] = h[5] + m[7] * two(sc)
                    for k, i in ((1, 0), (4, 7)):
                        h[k] = _cat([hold(h[k][e:e + 8], m[i][e:e + 8]) for e in (0, 8)], 0)
                    o = [pltpu.bitcast(q * jnp.tanh(q) + q, U32) + jnp.uint32(0x8000) for q in h]
                    for p in range(3):
                        words = (o[2 * p] >> 16) | (o[2 * p + 1] & jnp.uint32(0xFFFF0000))
                        for par in range(2):
                            os32[c, pl.ds(3 * (m0 + r0 + par) + p, 8, stride=6), :] = words[8 * par:8 * par + 8]

            def u_load(i, k0, k1, j0, j1):
                if i in (0, 7):
                    return wl[0 if i == 0 else 2, k0 * 128:k1 * 128, j0 * 128:j1 * 128]
                return _bf(_cat([_cat([u_low(j, k)[0].bitcast(U32)[u_low(j, k)[1], i - 1] for k in range(k0, k1)], 0)
                                 for j in range(j0, j1)], 1))

            def v_load(ch, i, k0, k1, m0, m1):
                return _bf(_cat([vs[ch][c].bitcast(U32)[i, m0 // 2:m1 // 2, :] for c in range(k0, k1)], 1))

            def rows8(r):
                return [(r, rr) for rr in range(0, r.shape[0], 8)]

            v0_bf16 = {}

            def dots_0(idx, m0, m1, j0, j1):
                gates = []
                for i in idx:
                    if m1 <= MA:
                        parts = [(p0, p1) for p0, p1 in ((0, MQ), (MQ, MA)) if m0 <= p0 < m1]
                        for p0, p1 in parts:
                            if (i, p0) not in v0_bf16:
                                v0_bf16[i, p0] = _cat(v_first[0][i][p0 // 8:p1 // 8], 0).astype(BF16)
                        lhs = _cat([v0_bf16[i, p0] for p0, _ in parts], 0)
                    else:
                        lhs = v_load(0, i, 0, 1, m0, m1)
                    r = _mm(lhs, u_load(i, 0, 1, j0, j1))
                    for j in range(j0, j1):
                        acc[j, i, m0:m1, :] = r[:, (j - j0) * 128:(j - j0 + 1) * 128]
                    gates += rows8(r)
                return gates

            def dots(ch, idx, k0, k1):
                gw = 4 // (k1 - k0)
                rows = slice(T0[ch], T0[ch] + MT[ch])
                gates = []
                for i in idx:
                    if k0 == 0:
                        lhs = _cat(v_first[ch][i], 0).astype(BF16)
                    else:
                        lhs = v_load(ch, i, k0, k1, 0, MT[ch])
                    for j in range(0, NC, gw):
                        r = _mm(lhs, u_load(i, k0, k1, j, j + gw))
                        if k0 > 0:
                            r = _cat([acc[j + q, i, rows, :] for q in range(gw)], 1) + r
                        for q in range(gw):
                            acc[j + q, i, rows, :] = r[:, q * 128:(q + 1) * 128]
                        gates += rows8(r)
                return gates

            with scope('w_w1'):
                wait(g_w1)
            with scope('W1'):
                start(g_b3)
                free(wl_items(range(2), 0, 1))
            with scope('w_x1'):
                wait(g_x1)
            x0 = x_items(0, [0])
            with scope('S1'):
                free(x0[:MQ // 16])
                dots_0(range(NP), 0, MQ, 0, 2)
            with scope('w_q'):
                wait(g_q)
            with scope('S2'):
                free(x0[MQ // 16:MA // 16])
                gt = dots_0((0, 7), 0, MQ, 2, 4) + dots_0(range(NP), MQ, MA, 0, 2)
                place(wl_items(range(2, 4), 0, 1), gt, 0.2, 0.8)
                dots_0((0, 7), MQ, MA, 2, 4)
                dots_0(range(1, 7), 0, MA, 2, 4)
            with scope('w_w2'):
                wait(g_w2)
            with scope('s0'):
                gt = dots_0((0, 7), 0, MA, 4, NC)
                free(x0[MA // 16:MA // 16 + 3])
                place(x0[MA // 16 + 3:], gt, 0.0, 0.2)
                gt += dots_0(range(NP), MA, MT[0], 0, 4)
                place(wl_items(range(4, NC), 0, 1), gt, 0.2, 0.9)
                dots_0((0, 7), MA, MT[0], 4, NC)
                for i in range(1, 7):
                    dots_0((i,), 0, MA, 4, NC), dots_0((i,), MA, MT[0], 4, NC)
            with scope('w_b2'):
                wait(g_b2)
            with scope('s1'):
                free(x_items(1, [0]))
                gt = dots(1, range(NP), 0, 1)
                place(x_items(0, [1]) + wl_items(range(NC), 1, 2), gt, 0.2, 0.95)
                dots(0, (0, 7, 1, 2, 3, 4), 1, 2)
                start(g_rest)
            with scope('w_b3'):
                wait(g_b3)
            with scope('s2'):
                gt = dots(0, (5, 6), 1, 2)
                place(x_items(1, [1]), gt, 0.0, 0.85)
                gt = dots(1, range(NP), 1, 2)
                place(x_items(0, [2, 3]) + wl_items(range(NC), 2, 4), gt, 0.0, 0.97)
                gt = dots(0, range(6), 2, 4)
                place(x_items(1, [2, 3]), gt, 0.0, 0.85)
            with scope('w_rest'):
                wait(g_rest)
            with scope('s3'):
                gt = dots(0, (6, 7), 2, 4) + dots(1, range(NP), 2, 4)
                place(x_items(0, range(4, NC)) + x_items(1, range(4, NC)) + wh_items(0, uh[0]), gt, 0.02, 0.98)
                mean_, var_, g_, b_ = (p[...].astype(F32).reshape(1, C) for p in (pm, pv, pg, pb))
                scale = g_ * jax.lax.rsqrt(var_ + 1e-5)
                for q, p in enumerate((0.5 * scale, 0.5 * (b_ - mean_ * scale))):
                    for j in range(NC):
                        bns[j, q] = jnp.broadcast_to(p[:, j * 128:(j + 1) * 128], (8, 128))

            def blocks(it, carry):
                views.clear()
                for jj in range(LB):
                    c = it * LB + jj
                    cuts = [0, MT[0]]
                    if jj == LB - 1:
                        cuts += [NT - 176, NT - 80, NT - 32]
                    gates = []
                    for t0, t1 in zip(cuts, cuts[1:] + [NT]):
                        ch = int(t0 >= T0[1])
                        M = [None] * NP
                        for i in (1, 2, 3, 4, 5, 6, 0, 7):
                            M[i] = acc[c, i, t0:t1, :] + _mm(v_load(ch, i, 4, NC, t0 - T0[ch], t1 - T0[ch]),
                                                             _bf(uh[jj % 2].bitcast(U32)[i]))
                            if i in (1, 2, 3) and t1 - t0 > 96:
                                gates += rows8(M[i])
                        epilogue(M, c, t0, t1)
                        send(c, t0, t1)
                    place(wh_items((c + 1) % NC, uh[(jj + 1) % 2]), gates, 0.0, 1.0)
                return carry
            with scope('B'):
                jax.lax.fori_loop(0, NC // LB, blocks, 0)
            with scope('w_out'):
                wait([orows(bb, c, 0, S) for bb in range(2) for c in range(NC)])

        vmem = pltpu.VMEM
        return pl.pallas_call(
            kern,
            in_specs=[pl.BlockSpec(memory_space=pl.ANY)] * 6,
            out_specs=pl.BlockSpec(memory_space=pl.ANY),
            out_shape=jax.ShapeDtypeStruct(x.shape, x.dtype),
            scratch_shapes=[
                vmem((NC, XR, 128), BF16), vmem((NC, OR, 128), BF16),
                vmem((3, KH, C), BF16), vmem((NC, 3, KH, 128), BF16),
                vmem((NC, NP, NT, 128), F32), vmem((NC, 2, 8, 128), F32),
                vmem((C,), BF16), vmem((C,), BF16), vmem((C,), BF16), vmem((C,), BF16),
                pltpu.SemaphoreType.DMA((6,)), pltpu.SemaphoreType.DMA((6,)),
                pltpu.SemaphoreType.DMA((1,)), pltpu.SemaphoreType.DMA((1,)),
                vmem((2, 6, 128, 128), BF16), vmem((2, 6, 128, 128), BF16), vmem((4, 6, 128, 128), BF16),
            ] + [vmem((NC, 6, 128, 128), BF16)] * 3 + [vmem((NP, KH, 128), BF16)] * 2
              + [vmem((NP, MT[0], 128), BF16)] * NC + [vmem((NP, MT[1], 128), BF16)] * NC,
            compiler_params=pltpu.CompilerParams(vmem_limit_bytes=110 * 2 ** 20, disable_bounds_checks=True,
                                                 disable_semaphore_checks=True),
        )(x, w, mean, var, g, b)
    return f


pallas_standalone__batchnorm__prompt_kernel = make()
```

```python
import contextlib
import functools

import jax
import jax.numpy as jnp
import jax.experimental.pallas as pl
import jax.experimental.pallas.tpu as pltpu

F32, U32, BF16 = jnp.float32, jnp.uint32, jnp.bfloat16

A = 0.52
B = 1.0 / A
A2, B2 = A * A, B * B
C1 = 1.0 / (2.0 * (1.0 - A2) * (1.0 - B2))
CA = 1.0 / (2.0 * A2 * (A2 - 1.0) * (A2 - B2))
CB = 1.0 / (2.0 * B2 * (B2 - 1.0) * (B2 - A2))
NP = 8


def _input_transform(d0, d1, d2, d3, d4, d5, d6, d7):
    d64, d42, d53, d31 = d6 - d4, d4 - d2, d5 - d3, d3 - d1
    v0 = (d0 - d6) + (A2 + 1.0 + B2) * d42
    v7 = (d7 - d1) - (A2 + 1.0 + B2) * d53
    e1 = (d6 + d2) - (A2 + B2) * d4
    o1 = (d5 + d1) - (A2 + B2) * d3
    ea, eb = d64 - B2 * d42, d64 - A2 * d42
    oa, ob = A * d53 - B * d31, B * d53 - A * d31
    return v0, e1 + o1, e1 - o1, ea + oa, ea - oa, eb + ob, eb - ob, v7


def _filter_transform(w0, w1, w2):
    e1, o1 = C1 * (w0 + w2), C1 * w1
    ea, oa = CA * w0 + (CA * A2) * w2, (CA * A) * w1
    eb, ob = CB * w0 + (CB * B2) * w2, (CB * B) * w1
    return e1 + o1, e1 - o1, ea + oa, ea - oa, eb + ob, eb - ob


def _bf(u):
    return pltpu.bitcast(u, BF16)


def _mm(a, b):
    return jnp.dot(a, b, preferred_element_type=F32)


def _cat(parts, axis):
    return parts[0] if len(parts) == 1 else jnp.concatenate(parts, axis=axis)


def make(scopes=False):
    scope = jax.named_scope if scopes else (lambda n: contextlib.nullcontext())

    @jax.jit
    def f(x, w, mean, var, g, b):
        _, S, C = x.shape
        assert x.shape == (2, 2048, 1024) and w.shape == (3, C, C)
        NC = C // 128
        KH = C // 2
        PADF, GAP = 16, 32
        B1 = S + GAP
        MT = (336, 352)
        T0 = (0, MT[0])
        NT = sum(MT)
        XR = PADF + 6 * NT + 32
        OR = 6 * NT + 16
        MQ, MA = 112, 208
        RQ, RA = 6 * MQ + 16, 6 * MA + 16
        LB = 4

        def kern(x_hbm, w_hbm, m_hbm, v_hbm, g_hbm, b_hbm, o_hbm,
                 xs, osb, wl, wh, acc, bns, pm, pv, pg, pb, xsem, wsem, osem, psem, *bufs):
            ul, uh = bufs[0:6], bufs[6:8]
            vs = (bufs[8:8 + NC], bufs[8 + NC:8 + 2 * NC])
            xs32, os32, wh32 = xs.bitcast(U32), osb.bitcast(U32), wh.bitcast(U32)

            def xrows(bb, c, r0, n, s):
                return pltpu.make_async_copy(x_hbm.at[bb, pl.ds(r0, n), pl.ds(c * 128, 128)],
                                             xs.at[c, pl.ds(PADF + bb * B1 + r0, n), :], xsem.at[s])

            def xcols(bb, cs, s):
                return [xrows(bb, c, 0, S, s) for c in cs]

            def wrows(k, s):
                return [pltpu.make_async_copy(w_hbm.at[:, pl.ds(k * 128, 128), :], wl.at[:, pl.ds(k * 128, 128), :],
                                              wsem.at[s])]

            def wpart(j0, j1, s):
                cols = pl.ds(j0 * 128, (j1 - j0) * 128)
                return [pltpu.make_async_copy(w_hbm.at[t, pl.ds(0, 128), cols], wl.at[t, pl.ds(0, 128), cols],
                                              wsem.at[s]) for t in range(3)]

            def whigh(s):
                return [pltpu.make_async_copy(w_hbm.at[t, pl.ds(KH, KH), pl.ds(j * 128, 128)], wh.at[j, t], wsem.at[s])
                        for j in range(NC) for t in range(3)]

            def orows(bb, c, r0, n):
                col = c * 128 if isinstance(c, int) else pl.multiple_of(c * 128, 128)
                return pltpu.make_async_copy(osb.at[c, pl.ds(bb * B1 + r0, n), :],
                                             o_hbm.at[bb, pl.ds(r0, n), pl.ds(col, 128)], osem.at[0])

            def send(c, t0, t1):
                for bb in range(2):
                    lo, hi = max(6 * t0, bb * B1), min(6 * t1, bb * B1 + S)
                    if hi > lo:
                        orows(bb, c, lo - bb * B1, hi - lo).start()

            def start(cs):
                for cp in cs:
                    cp.start()

            def wait(cs):
                for cp in cs:
                    cp.wait()

            g_w1 = wpart(0, 2, 0)
            g_x1 = [xrows(0, 0, 0, RQ, 0)]
            g_q = wpart(2, 4, 1) + [xrows(0, 0, RQ, RA - RQ, 1)]
            g_w2 = wpart(4, NC, 2) + [xrows(0, 0, RA, S - RA, 2)]
            g_b2 = xcols(1, [0], 3) + xcols(0, [1], 3) + wrows(1, 3)
            g_b3 = xcols(1, [1, 2, 3], 4) + xcols(0, [2, 3], 4) + wrows(2, 4) + wrows(3, 4)
            g_rest = xcols(0, range(4, NC), 5) + xcols(1, range(4, NC), 5) + whigh(5) + [
                pltpu.make_async_copy(src, dst, psem.at[0])
                for src, dst in ((m_hbm, pm), (v_hbm, pv), (g_hbm, pg), (b_hbm, pb))]

            def runtime_zero(seed):
                return jax.lax.fori_loop(0, 5, lambda i, c: c >> 1, seed)

            zero = 0
            for n, group in enumerate((g_w1, g_x1, g_q, g_w2)):
                start(group)
                zero = zero + runtime_zero(17 + 2 * n)
            start(g_b2)
            for c in range(NC):
                for r0, r1 in ((0, PADF), (PADF + S, PADF + B1), (PADF + B1 + S, XR)):
                    xs[c, pl.ds(r0, r1 - r0), :] = jnp.zeros((r1 - r0, 128), BF16)

            views = {}

            def shifted(buf):
                if id(buf) not in views:
                    rows = pl.ds(pl.multiple_of(zero, 16), buf.shape[-2])
                    views[id(buf)] = buf.at[(slice(None),) * (len(buf.shape) - 2) + (rows, slice(None))]
                return views[id(buf)]

            true = jnp.full((8, 128), zero, jnp.int32) == 0

            def hold(v, gate):
                return jax.lax.select(true, v, gate if gate.dtype == v.dtype else pltpu.bitcast(gate, v.dtype))

            def place(items, gates, f0, f1):
                for k, item in enumerate(items):
                    gi = int(len(gates) * (f0 + (f1 - f0) * k / len(items)))

                    @functools.cache
                    def gate(d, gi=gi):
                        arr, r = gates[min(gi + d, len(gates) - 1)]
                        return pltpu.bitcast(arr[r:r + 8, 0:128], U32)
                    item(gate)

            def free(items):
                for item in items:
                    item(None)

            def u_low(j, k):
                if k > 0:
                    return ul[2 + k], j
                return (ul[0], j) if j < 2 else (ul[1], j - 2) if j < 4 else (ul[2], j - 4)

            def filter16(raw, gate):
                if gate is None:
                    return _filter_transform(*(_bf(u).astype(F32) for u in raw))
                top = _filter_transform(*(_bf(hold(u, gate(0))).astype(F32)[0:8] for u in raw))
                bot = _filter_transform(*(_bf(hold(u, gate(2))).astype(F32)[8:16] for u in raw))
                return [_cat(p, 0) for p in zip(top, bot)]

            def wl_item(j, r0, gate):
                raw = [pltpu.bitcast(wl[t, pl.ds(r0, 16), pl.ds(j * 128, 128)], U32) for t in range(3)]
                buf, slot = u_low(j, r0 // 128)
                for i, u in enumerate(filter16(raw, gate)):
                    shifted(buf)[slot, i, pl.ds(r0 % 128, 16), :] = u.astype(BF16)

            def wl_items(js, k0, k1):
                return [functools.partial(wl_item, j, r0) for j in js for r0 in range(k0 * 128, k1 * 128, 16)]

            def wh_item(j, buf, r0, gate):
                raw = [wh32[j, t, pl.ds(r0 // 2, 8), :] for t in range(3)]
                us = [u.astype(BF16) for u in filter16(raw, gate)]
                for i, u in enumerate([_bf(hold(raw[0], gate(0)))] + us + [_bf(hold(raw[2], gate(0)))]):
                    shifted(buf)[i, pl.ds(r0, 16), :] = u

            def wh_items(j, buf):
                return [functools.partial(wh_item, j, buf, r0) for r0 in range(0, KH, 16)]

            high, sixteen = jnp.full((8, 128), 0xFFFF0000, U32), jnp.full((8, 128), 16, U32)

            def unpackers(gate, d):
                mask, shift = high, sixteen
                if gate is not None:
                    mask, shift = hold(mask, gate(d)), hold(shift, gate(d))
                return (lambda u: pltpu.bitcast(u << shift, F32)), (lambda u: pltpu.bitcast(u & mask, F32))

            v_first = [[[] for _ in range(NP)] for _ in range(2)]

            def x_item(ch, c, t0, gate):
                base = PADF // 2 + 3 * (T0[ch] + t0)
                u = [xs32[c, pl.ds(base + o, 8, stride=6), :] for o in range(-1, 7)]
                lo, hi = unpackers(gate, 0)
                d = [hi(u[0]), lo(u[1]), hi(u[1]), lo(u[2]), hi(u[2]), lo(u[3]), hi(u[3]), lo(u[4])]
                lo, hi = unpackers(gate, 2)
                d += [hi(u[4]), lo(u[5]), hi(u[5]), lo(u[6]), hi(u[6]), lo(u[7])]
                even, odd = _input_transform(*d[0:8]), _input_transform(*d[6:14])
                for i in range(NP):
                    if c == 0 and (ch == 1 or t0 < MA):
                        v_first[ch][i] += [even[i], odd[i]]
                    else:
                        shifted(vs[ch][c])[i, pl.ds(t0, 16), :] = _cat([even[i], odd[i]], 0).astype(BF16)

            def x_items(ch, cs):
                return [functools.partial(x_item, ch, c, t0) for c in cs for t0 in range(0, MT[ch], 16)]

            def epilogue(M, c, m0, m1):
                sc, sh = bns[c, 0], bns[c, 1]
                ka, kb = [A ** k * sc for k in range(6)], [B ** k * sc for k in range(6)]

                def two(v):
                    return _cat([v, v], 0)
                for r0 in range(0, m1 - m0, 16):
                    m = [q[r0:r0 + 16] for q in M]
                    p1 = ((m[1] + m[2]) * two(sc) + two(sh), (m[1] - m[2]) * two(sc) + two(sh))
                    pa, pb_ = (m[3] + m[4], m[3] - m[4]), (m[5] + m[6], m[5] - m[6])
                    kk = [two(hold(ka[k], m[5][0:8]) if k % 2 else ka[k]) for k in range(6)]
                    h = [(p1[k % 2] + pa[k % 2] * kk[k]) + pb_[k % 2] * two(kb[k]) for k in range(6)]
                    h[0] = h[0] + m[0] * two(sc)
                    h[5] = h[5] + m[7] * two(sc)
                    for k, i in ((1, 0), (4, 7)):
                        h[k] = _cat([hold(h[k][e:e + 8], m[i][e:e + 8]) for e in (0, 8)], 0)
                    o = [pltpu.bitcast(q * jnp.tanh(q) + q, U32) + jnp.uint32(0x8000) for q in h]
                    for p in range(3):
                        words = (o[2 * p] >> 16) | (o[2 * p + 1] & jnp.uint32(0xFFFF0000))
                        for par in range(2):
                            os32[c, pl.ds(3 * (m0 + r0 + par) + p, 8, stride=6), :] = words[8 * par:8 * par + 8]

            def u_load(i, k0, k1, j0, j1):
                if i in (0, 7):
                    return wl[0 if i == 0 else 2, k0 * 128:k1 * 128, j0 * 128:j1 * 128]
                return _bf(_cat([_cat([u_low(j, k)[0].bitcast(U32)[u_low(j, k)[1], i - 1] for k in range(k0, k1)], 0)
                                 for j in range(j0, j1)], 1))

            def v_load(ch, i, k0, k1, m0, m1):
                return _bf(_cat([vs[ch][c].bitcast(U32)[i, m0 // 2:m1 // 2, :] for c in range(k0, k1)], 1))

            def rows8(r):
                return [(r, rr) for rr in range(0, r.shape[0], 8)]

            v0_bf16 = {}

            def dots_0(idx, m0, m1, j0, j1):
                gates = []
                for i in idx:
                    if m1 <= MA:
                        parts = [(p0, p1) for p0, p1 in ((0, MQ), (MQ, MA)) if m0 <= p0 < m1]
                        for p0, p1 in parts:
                            if (i, p0) not in v0_bf16:
                                v0_bf16[i, p0] = _cat(v_first[0][i][p0 // 8:p1 // 8], 0).astype(BF16)
                        lhs = _cat([v0_bf16[i, p0] for p0, _ in parts], 0)
                    else:
                        lhs = v_load(0, i, 0, 1, m0, m1)
                    r = _mm(lhs, u_load(i, 0, 1, j0, j1))
                    for j in range(j0, j1):
                        acc[j, i, m0:m1, :] = r[:, (j - j0) * 128:(j - j0 + 1) * 128]
                    gates += rows8(r)
                return gates

            def dots(ch, idx, k0, k1):
                gw = 4 // (k1 - k0)
                rows = slice(T0[ch], T0[ch] + MT[ch])
                gates = []
                for i in idx:
                    if k0 == 0:
                        lhs = _cat(v_first[ch][i], 0).astype(BF16)
                    else:
                        lhs = v_load(ch, i, k0, k1, 0, MT[ch])
                    for j in range(0, NC, gw):
                        r = _mm(lhs, u_load(i, k0, k1, j, j + gw))
                        if k0 > 0:
                            r = _cat([acc[j + q, i, rows, :] for q in range(gw)], 1) + r
                        for q in range(gw):
                            acc[j + q, i, rows, :] = r[:, q * 128:(q + 1) * 128]
                        gates += rows8(r)
                return gates

            with scope('w_w1'):
                wait(g_w1)
            with scope('W1'):
                start(g_b3)
                free(wl_items(range(2), 0, 1))
            with scope('w_x1'):
                wait(g_x1)
            x0 = x_items(0, [0])
            with scope('S1'):
                free(x0[:MQ // 16])
                dots_0(range(NP), 0, MQ, 0, 2)
            with scope('w_q'):
                wait(g_q)
            with scope('S2'):
                free(x0[MQ // 16:MA // 16])
                gt = dots_0((0, 7), 0, MQ, 2, 4) + dots_0(range(NP), MQ, MA, 0, 2)
                place(wl_items(range(2, 4), 0, 1), gt, 0.2, 0.8)
                dots_0((0, 7), MQ, MA, 2, 4)
                dots_0(range(1, 7), 0, MA, 2, 4)
            with scope('w_w2'):
                wait(g_w2)
            with scope('s0'):
                gt = dots_0((0, 7), 0, MA, 4, NC)
                free(x0[MA // 16:MA // 16 + 3])
                place(x0[MA // 16 + 3:], gt, 0.0, 0.2)
                gt += dots_0(range(NP), MA, MT[0], 0, 4)
                place(wl_items(range(4, NC), 0, 1), gt, 0.2, 0.9)
                dots_0((0, 7), MA, MT[0], 4, NC)
                for i in range(1, 7):
                    dots_0((i,), 0, MA, 4, NC), dots_0((i,), MA, MT[0], 4, NC)
            with scope('w_b2'):
                wait(g_b2)
            with scope('s1'):
                free(x_items(1, [0]))
                gt = dots(1, range(NP), 0, 1)
                place(x_items(0, [1]) + wl_items(range(NC), 1, 2), gt, 0.2, 0.95)
                dots(0, (0, 7, 1, 2, 3, 4), 1, 2)
                start(g_rest)
            with scope('w_b3'):
                wait(g_b3)
            with scope('s2'):
                gt = dots(0, (5, 6), 1, 2)
                place(x_items(1, [1]), gt, 0.0, 0.85)
                gt = dots(1, range(NP), 1, 2)
                place(x_items(0, [2, 3]) + wl_items(range(NC), 2, 4), gt, 0.0, 0.97)
                gt = dots(0, range(6), 2, 4)
                place(x_items(1, [2, 3]), gt, 0.0, 0.85)
            with scope('w_rest'):
                wait(g_rest)
            with scope('s3'):
                gt = dots(0, (6, 7), 2, 4) + dots(1, range(NP), 2, 4)
                place(x_items(0, range(4, NC)) + x_items(1, range(4, NC)) + wh_items(0, uh[0]), gt, 0.02, 0.98)
                mean_, var_, g_, b_ = (p[...].astype(F32).reshape(1, C) for p in (pm, pv, pg, pb))
                scale = g_ * jax.lax.rsqrt(var_ + 1e-5)
                for q, p in enumerate((0.5 * scale, 0.5 * (b_ - mean_ * scale))):
                    for j in range(NC):
                        bns[j, q] = jnp.broadcast_to(p[:, j * 128:(j + 1) * 128], (8, 128))

            def blocks(it, carry):
                views.clear()
                for jj in range(LB):
                    c = it * LB + jj
                    cuts = [0, MT[0]]
                    if jj == LB - 1:
                        cuts += [NT - 176, NT - 80, NT - 32]
                    gates = []
                    for t0, t1 in zip(cuts, cuts[1:] + [NT]):
                        ch = int(t0 >= T0[1])
                        M = [None] * NP
                        for i in (1, 2, 3, 4, 5, 6, 0, 7):
                            M[i] = acc[c, i, t0:t1, :] + _mm(v_load(ch, i, 4, NC, t0 - T0[ch], t1 - T0[ch]),
                                                             _bf(uh[jj % 2].bitcast(U32)[i]))
                            if i in (1, 2, 3) and t1 - t0 > 96:
                                gates += rows8(M[i])
                        epilogue(M, c, t0, t1)
                        send(c, t0, t1)
                    place(wh_items((c + 1) % NC, uh[(jj + 1) % 2]), gates, 0.0, 1.0)
                return carry
            with scope('B'):
                jax.lax.fori_loop(0, NC // LB, blocks, 0)
            with scope('w_out'):
                wait([orows(bb, c, 0, S) for bb in range(2) for c in range(NC)])

        vmem = pltpu.VMEM
        return pl.pallas_call(
            kern,
            in_specs=[pl.BlockSpec(memory_space=pl.ANY)] * 6,
            out_specs=pl.BlockSpec(memory_space=pl.ANY),
            out_shape=jax.ShapeDtypeStruct(x.shape, x.dtype),
            scratch_shapes=[
                vmem((NC, XR, 128), BF16), vmem((NC, OR, 128), BF16),
                vmem((3, KH, C), BF16), vmem((NC, 3, KH, 128), BF16),
                vmem((NC, NP, NT, 128), F32), vmem((NC, 2, 8, 128), F32),
                vmem((C,), BF16), vmem((C,), BF16), vmem((C,), BF16), vmem((C,), BF16),
                pltpu.SemaphoreType.DMA((6,)), pltpu.SemaphoreType.DMA((6,)),
                pltpu.SemaphoreType.DMA((1,)), pltpu.SemaphoreType.DMA((1,)),
                vmem((2, 6, 128, 128), BF16), vmem((2, 6, 128, 128), BF16), vmem((4, 6, 128, 128), BF16),
            ] + [vmem((NC, 6, 128, 128), BF16)] * 3 + [vmem((NP, KH, 128), BF16)] * 2
              + [vmem((NP, MT[0], 128), BF16)] * NC + [vmem((NP, MT[1], 128), BF16)] * NC,
            compiler_params=pltpu.CompilerParams(vmem_limit_bytes=110 * 2 ** 20, disable_bounds_checks=True,
                                                 disable_semaphore_checks=True),
        )(x, w, mean, var, g, b)
    return f


pallas_standalone__batchnorm__prompt_kernel = make()
```
